```python
import jax
import jax.numpy as jnp

def _softmax(x, axis=-1):
    return jax.nn.softmax(x, axis=axis)

def _gelu(x):
    return jax.nn.gelu(x, approximate=True)

def _silu(x):
    return jax.nn.silu(x)

def _sigmoid(x):
    return jax.nn.sigmoid(x)

def _layernorm(x, axis=-1, eps=1e-05):
    m = jnp.mean(x, axis=axis, keepdims=True)
    v = jnp.var(x, axis=axis, keepdims=True)
    return (x - m) / jnp.sqrt(v + eps)

def _scatter_add(tgt, idx, src, axis=0):
    return tgt.at[idx].add(src)

def _segment_sum(src, seg, n):
    return jax.ops.segment_sum(src, seg, n)

class _Rng:

    def __init__(self, key):
        self._k = key

    def _next(self):
        self._k, sub = jax.random.split(self._k)
        return sub

    def normal(self, shape):
        return jax.random.normal(self._next(), shape, dtype=jnp.bfloat16)

    def randint(self, lo, hi, shape):
        return jax.random.randint(self._next(), shape, lo, hi, dtype=jnp.int32)

    def uniform(self, shape, lo=0.0, hi=1.0):
        return jax.random.uniform(self._next(), shape, jnp.bfloat16, lo, hi)

    def permutation(self, n):
        return jax.random.permutation(self._next(), n)
kernel_name = 'standalone__conformer_family_branchformer__speech'

def setup_inputs():
    _rng = _Rng(jax.random.key(int.from_bytes(__import__("os").urandom(4), "little")))
    _w = lambda a: (lambda t: t.astype(jnp.bfloat16) if jnp.issubdtype(t.dtype, jnp.floating) else t)(jnp.asarray(a))
    B, T, D, K = (2, 4000, 512, 31)
    s = float(D) ** (-0.5)
    return {'x': _w((lambda *s: _rng.normal(s) * 0.05)(B, T, D)), 'w_q': _w((lambda *s: _rng.normal(s) * 0.05)(D, D) * s), 'w_k': _w((lambda *s: _rng.normal(s) * 0.05)(D, D) * s), 'w_v': _w((lambda *s: _rng.normal(s) * 0.05)(D, D) * s), 'w_ao': _w((lambda *s: _rng.normal(s) * 0.05)(D, D) * s), 'w_up': _w((lambda *s: _rng.normal(s) * 0.05)(D, 2 * D) * s), 'dw': _w((lambda *s: _rng.normal(s) * 0.05)(K, D) * (1.0 / K)), 'w_dn': _w((lambda *s: _rng.normal(s) * 0.05)(D, D) * s), 'w_merge': _w((lambda *s: _rng.normal(s) * 0.05)(2 * D, D) * s)}

def reference(x, w_q, w_k, w_v, w_ao, w_up, dw, w_dn, w_merge):
    B, T, D = x.shape
    K = dw.shape[0]
    xa = _layernorm(x, axis=-1)
    q = jnp.einsum('btd,de->bte', xa, w_q)
    k = jnp.einsum('btd,de->bte', xa, w_k)
    v = jnp.einsum('btd,de->bte', xa, w_v)
    logits = jnp.einsum('btd,bsd->bts', q, k) * float(D) ** (-0.5)
    attn = _softmax(logits, axis=-1)
    ya = jnp.einsum('bts,bsd->btd', attn, v)
    ya = jnp.einsum('btd,de->bte', ya, w_ao)
    xc = _layernorm(x, axis=-1)
    h = _gelu(jnp.einsum('btd,de->bte', xc, w_up))
    u = h[..., :D].copy()
    g = _layernorm(h[..., D:], axis=-1)
    pad = K // 2
    gp = jnp.pad(g, ((0, 0), (pad, pad), (0, 0)))
    conv = jnp.zeros_like(g)
    for i in range(K):
        conv = conv + gp[:, i:i + T, :] * dw[i][None, None, :]
    yc = jnp.einsum('btd,de->bte', u * conv, w_dn)
    merged = jnp.concatenate([ya, yc], axis=-1)
    out = jnp.einsum('btf,fd->btd', merged, w_merge)
    return x + out
```

```python
import math
import jax
import jax.numpy as jnp
from jax import lax
import jax.experimental.pallas as pl
import jax.experimental.pallas.tpu as pltpu

TQ = 400
KC = 512
RB = 16
GPT = 4
AHEAD = 1
PR = 48
FLAGS = None
F32 = jnp.float32
BF16 = jnp.bfloat16


def _dot(a, b):
    return jnp.dot(a, b, preferred_element_type=F32)


def _dot_nt(a, b):
    return lax.dot_general(a, b, (((1,), (1,)), ((), ())), preferred_element_type=F32)


def _ln(x):
    m = jnp.mean(x, axis=-1, keepdims=True)
    xc = x - m
    v = jnp.mean(xc * xc, axis=-1, keepdims=True)
    return xc * lax.rsqrt(v + 1e-5)


def _gelu(x):
    c = math.sqrt(2.0 / math.pi)
    hx = 0.5 * x
    return hx + hx * jnp.tanh(x * (c + (c * 0.044715) * (x * x)))


@jax.jit
def pallas_standalone__conformer_family_branchformer__speech_kernel(
    x, w_q, w_k, w_v, w_ao, w_up, dw, w_dn, w_merge,
):
    B, T, D = x.shape
    K = dw.shape[0]
    tq = TQ
    nq = T // tq
    TP = (T + KC - 1) // KC * KC
    nkc = TP // KC
    HALO = 16
    NL = D // 128
    PC = 512
    TPC = KC // 128

    def kernel(x_ref, wq_ref, wk_ref, wv_ref, wao_ref, wup_ref, dw_ref, wdn_ref, wm_ref, o_ref,
               m_s, wvo_s, wdm_s, dwb_s, xa_s, v_s, g_s, u_s, z_s, s_s):
        b = pl.program_id(0)
        i = pl.program_id(1)

        @pl.when((b == 0) & (i == 0))
        def _():
            sc = float(D) ** -0.5 * math.log2(math.e)
            m_s[...] = (_dot_nt(wq_ref[...], wk_ref[...]) * sc).astype(BF16)
            t = _dot(wao_ref[...], wm_ref[0:D, :]).astype(BF16)
            wvo_s[...] = _dot(wv_ref[...], t).astype(BF16)
            wdm_s[...] = _dot(wdn_ref[...], wm_ref[D:2 * D, :]).astype(BF16)
            xa_s[T:, :] = jnp.zeros((xa_s.shape[0] - T, D), BF16)
            dwf = dw_ref[...].astype(F32)
            for k in range(K):
                dwb_s[k] = jnp.broadcast_to(dwf[k:k + 1, :], (8, D))

        @pl.when(i == 0)
        def _():
            for c in range(TP // PC):
                r0 = c * PC
                n = min(PC, T - r0)
                xa = _ln(x_ref[0, r0:r0 + n, :].astype(F32)).astype(BF16)
                xa_s[r0:r0 + n, :] = xa
                full = xa_s[r0:r0 + PC, :]
                v_s[r0:r0 + PC, :] = _dot(full, wvo_s[...]).astype(BF16)
            g0 = _ln(_gelu(_dot(xa_s[0:tq + HALO, :], wup_ref[:, D:2 * D])))
            for j in range(NL):
                g_s[j, 0:HALO, :] = jnp.zeros((HALO, 128), F32)
                g_s[j, HALO:tq + 2 * HALO, :] = g0[:, j * 128:(j + 1) * 128]

        r0 = pl.multiple_of(i * tq, 16)
        xq = xa_s[pl.ds(r0, tq), :]
        q = _dot(xq, m_s[...]).astype(BF16)
        u_s[...] = _gelu(_dot(xq, wup_ref[:, 0:D]))

        pieces = [(a, min(RB, tq - a), j) for a in range(0, tq, RB) for j in range(NL)]
        spare_g = pl.multiple_of(tq + 2 * HALO + 8 * b, 8)
        spare_s = pl.multiple_of(tq + 8 * b, 8)

        def conv_piece(a, n, j, gate):
            g_s[j, pl.ds(spare_g, 8), :] = gate
            acc = None
            for k in sorted(range(K), key=lambda k: (k % 8, k)):
                w = dwb_s[k, :, j * 128:(j + 1) * 128]
                t = g_s[j, a + k + 1:a + k + 1 + n, :].reshape(n // 8, 8, 128) * w[None]
                acc = t if acc is None else acc + t
            conv = acc.reshape(n, 128)
            z_s[a:a + n, j * 128:(j + 1) * 128] = (conv * u_s[a:a + n, j * 128:(j + 1) * 128]).astype(BF16)

        mx = None
        for c in range(nkc):
            s = _dot_nt(q, xa_s[c * KC:(c + 1) * KC, :])
            for j in range(TPC):
                kt = c * TPC + j
                t = s[:, j * 128:(j + 1) * 128]
                if (kt + 1) * 128 > T:
                    col = kt * 128 + lax.broadcasted_iota(jnp.int32, (tq, 128), 1)
                    t = jnp.where(col < T, t, -jnp.inf)
                s_s[kt, 0:tq, :] = t
                mx = t if mx is None else jnp.maximum(mx, t)
                for rr in range(GPT):
                    if pieces:
                        r = (tq // GPT * rr) // 8 * 8
                        conv_piece(*pieces.pop(0), t[r:r + 8, :])
        assert not pieces
        m = jnp.max(mx, axis=-1, keepdims=True)

        rn = jnp.minimum(r0 + tq + HALO, TP - tq)
        xg = xa_s[pl.ds(pl.multiple_of(rn, 16), tq), :]
        g = _ln(_gelu(_dot(xg, wup_ref[:, D:2 * D])))
        row = rn + lax.broadcasted_iota(jnp.int32, (tq, D), 0)
        g = jnp.where(row < T, g, 0.0)
        for j in range(NL):
            g_s[j, 0:2 * HALO, :] = g_s[j, tq:tq + 2 * HALO, :]
            g_s[j, 2 * HALO:tq + 2 * HALO, :] = g[:, j * 128:(j + 1) * 128]
        oc = _dot(z_s[...], wdm_s[...]) + x_ref[0, pl.ds(r0, tq), :].astype(F32)

        rblocks = [(a, min(PR, tq - a)) for a in range(0, tq, PR)]
        ls = {}
        pblk = {}

        def exp_piece(c, a, n, gate):
            if gate is not None:
                s_s[0, pl.ds(spare_s, 8), :] = gate
            mm = m[a:a + n]
            ps = None
            tiles = []
            for j in range(TPC):
                p = jnp.exp2(s_s[c * TPC + j, a:a + n, :] - mm)
                ps = p if ps is None else ps + p
                tiles.append(p.astype(BF16))
            ls[a] = ps if a not in ls else ls[a] + ps
            pblk[c, a] = jnp.concatenate(tiles, axis=1)

        for c in range(AHEAD):
            for a, n in rblocks:
                exp_piece(c, a, n, None)
        acc = None
        for c in range(nkc):
            p = jnp.concatenate([pblk.pop((c, a)) for a, n in rblocks], axis=0)
            pv = _dot(p, v_s[c * KC:(c + 1) * KC, :])
            acc = pv if acc is None else acc + pv
            if c + AHEAD < nkc:
                for ib, (a, n) in enumerate(rblocks):
                    pos = ib * NL * tq // len(rblocks)
                    jj = pos // tq
                    r = (pos % tq) // 8 * 8
                    exp_piece(c + AHEAD, a, n, acc[r:r + 8, jj * 128:(jj + 1) * 128])
        ls = [jnp.concatenate([ls[a] for a, n in rblocks], axis=0)]
        l = jnp.sum(ls[0], axis=-1, keepdims=True)
        out = acc * (1.0 / l) + oc
        o_ref[0] = out.astype(o_ref.dtype)

    def full(a):
        return pl.BlockSpec(a.shape, lambda b, i: (0,) * a.ndim)

    return pl.pallas_call(
        kernel,
        grid=(B, nq),
        in_specs=[pl.BlockSpec((1, T, D), lambda b, i: (b, 0, 0))] + [full(a) for a in (w_q, w_k, w_v, w_ao, w_up, dw, w_dn, w_merge)],
        out_specs=pl.BlockSpec((1, tq, D), lambda b, i: (b, i, 0)),
        out_shape=jax.ShapeDtypeStruct((B, T, D), x.dtype),
        scratch_shapes=[
            pltpu.VMEM((D, D), BF16), pltpu.VMEM((D, D), BF16), pltpu.VMEM((D, D), BF16),
            pltpu.VMEM((K, 8, D), F32),
            pltpu.VMEM((TP, D), BF16), pltpu.VMEM((TP, D), BF16),
            pltpu.VMEM((NL, tq + 2 * HALO + 16, 128), F32), pltpu.VMEM((tq, D), F32), pltpu.VMEM((tq, D), BF16),
            pltpu.VMEM((TP // 128, tq + 16, 128), F32),
        ],
        compiler_params=pltpu.CompilerParams(
            dimension_semantics=("arbitrary", "arbitrary"),
            vmem_limit_bytes=100 * 1024 * 1024, flags=FLAGS,
        ),
    )(x, w_q, w_k, w_v, w_ao, w_up, dw, w_dn, w_merge)
```

```python
import math
import jax
import jax.numpy as jnp
from jax import lax
import jax.experimental.pallas as pl
import jax.experimental.pallas.tpu as pltpu

TQ = 400
KC = 512
RB = 16
G0 = 6
G1 = 32
AHEAD = 1
PR = 48
FLAGS = None
F32 = jnp.float32
BF16 = jnp.bfloat16


def _dot(a, b):
    return jnp.dot(a, b, preferred_element_type=F32)


def _dot_nt(a, b):
    return lax.dot_general(a, b, (((1,), (1,)), ((), ())), preferred_element_type=F32)


def _ln(x):
    m = jnp.mean(x, axis=-1, keepdims=True)
    xc = x - m
    v = jnp.mean(xc * xc, axis=-1, keepdims=True)
    return xc * lax.rsqrt(v + 1e-5)


def _gelu(x):
    c = math.sqrt(2.0 / math.pi)
    hx = 0.5 * x
    return hx + hx * jnp.tanh(x * (c + (c * 0.044715) * (x * x)))


@jax.jit
def pallas_standalone__conformer_family_branchformer__speech_kernel(
    x, w_q, w_k, w_v, w_ao, w_up, dw, w_dn, w_merge,
):
    B, T, D = x.shape
    K = dw.shape[0]
    tq = TQ
    nq = T // tq
    TP = (T + KC - 1) // KC * KC
    nkc = TP // KC
    HALO = 16
    NL = D // 128
    TPC = KC // 128
    XH = 2048

    def kernel(x_hbm, wq_hbm, wk_hbm, wv_hbm, wao_hbm, wup_hbm, dw_hbm, wdn_hbm, wm_hbm, o_ref,
               x_s, wq_s, wk_s, wv_s, wao_s, wup_s, dw_s, wdn_s, wm_s, wsem, xsem,
               m_s, wvo_s, wdm_s, dwb_s, xa_s, v_s, g_s, u_s, z_s, s_s):
        b = pl.program_id(0)
        i = pl.program_id(1)

        def x_copy(bb, h):
            rows = pl.ds(0, XH) if h == 0 else pl.ds(XH, T - XH)
            return pltpu.make_async_copy(x_hbm.at[bb, rows], x_s.at[bb, rows], xsem.at[2 * bb + h])

        @pl.when((b == 0) & (i == 0))
        def _():
            top, bot = pl.ds(0, D), pl.ds(D, D)
            cp = [pltpu.make_async_copy(s, d, wsem.at[n]) for n, (s, d) in enumerate([
                (wao_hbm, wao_s), (wm_hbm.at[top], wm_s.at[top]), (wv_hbm, wv_s),
                (wq_hbm, wq_s), (wk_hbm, wk_s), (wdn_hbm, wdn_s), (wm_hbm.at[bot], wm_s.at[bot]),
                (dw_hbm, dw_s), (wup_hbm, wup_s)])]
            cp[0].start(); cp[1].start(); cp[2].start()
            xa_s[T:, :] = jnp.zeros((TP - T, D), BF16)
            v_s[T:, :] = jnp.zeros((TP - T, D), BF16)
            cp[0].wait(); cp[1].wait()
            cp[3].start(); cp[4].start()
            t = _dot(wao_s[...], wm_s[0:D, :]).astype(BF16)
            cp[2].wait()
            cp[5].start(); cp[6].start(); cp[7].start()
            wvo_s[...] = _dot(wv_s[...], t).astype(BF16)
            cp[3].wait(); cp[4].wait()
            x_copy(0, 0).start()
            sc = float(D) ** -0.5 * math.log2(math.e)
            m_s[...] = (_dot_nt(wq_s[...], wk_s[...]) * sc).astype(BF16)
            cp[5].wait(); cp[6].wait(); cp[7].wait()
            cp[8].start()
            x_copy(0, 1).start()
            wdm_s[...] = _dot(wdn_s[...], wm_s[D:2 * D, :]).astype(BF16)
            dwf = dw_s[...].astype(F32)
            for k in range(K):
                dwb_s[k] = jnp.broadcast_to(dwf[k:k + 1, :], (8, D))
            cp[8].wait()
            for bb in range(1, B):
                x_copy(bb, 0).start()
                x_copy(bb, 1).start()

        @pl.when(i == 0)
        def _():
            def rows(r0, n):
                xa = _ln(x_s[b, r0:r0 + n, :].astype(F32)).astype(BF16)
                xa_s[r0:r0 + n, :] = xa
                v_s[r0:r0 + n, :] = _dot(xa, wvo_s[...]).astype(BF16)

            x_copy(b, 0).wait()
            for r0, n in ((0, 128), (128, 384), (512, 512), (1024, 512), (1536, 512)):
                rows(r0, n)
            g0 = _ln(_gelu(_dot(xa_s[0:HALO, :], wup_s[:, D:2 * D])))
            for j in range(NL):
                g_s[j, tq:tq + HALO, :] = jnp.zeros((HALO, 128), F32)
                g_s[j, tq + HALO:tq + 2 * HALO, :] = g0[:, j * 128:(j + 1) * 128]
            x_copy(b, 1).wait()
            for r0 in range(XH, T, 512):
                rows(r0, min(512, T - r0))

        r0 = pl.multiple_of(i * tq, 16)
        xq = xa_s[pl.ds(r0, tq), :]
        xg = xa_s[pl.ds(pl.multiple_of(r0 + HALO, 16), tq), :]
        g = _ln(_gelu(_dot(xg, wup_s[:, D:2 * D])))
        for j in range(NL):
            g_s[j, 0:2 * HALO, :] = g_s[j, tq:tq + 2 * HALO, :]
            g_s[j, 2 * HALO:tq + 2 * HALO, :] = g[:, j * 128:(j + 1) * 128]
        u_s[...] = _gelu(_dot(xq, wup_s[:, 0:D]))
        q = _dot(xq, m_s[...]).astype(BF16)

        pieces = [(a, min(RB, tq - a), j) for a in range(0, tq, RB) for j in range(NL)]
        npieces = len(pieces)
        spare_g = pl.multiple_of(tq + 2 * HALO + 8 * b, 8)
        spare_s = pl.multiple_of(tq + 8 * b, 8)

        def conv_piece(a, n, j, gate):
            g_s[j, pl.ds(spare_g, 8), :] = gate
            acc = None
            for k in sorted(range(K), key=lambda k: (k % 8, k)):
                w = dwb_s[k, :, j * 128:(j + 1) * 128]
                t = g_s[j, a + k + 1:a + k + 1 + n, :].reshape(n // 8, 8, 128) * w[None]
                acc = t if acc is None else acc + t
            conv = acc.reshape(n, 128)
            z_s[a:a + n, j * 128:(j + 1) * 128] = (conv * u_s[a:a + n, j * 128:(j + 1) * 128]).astype(BF16)

        mx = None
        for c in range(nkc):
            s = _dot_nt(q, xa_s[c * KC:(c + 1) * KC, :])
            for j in range(TPC):
                kt = c * TPC + j
                t = s[:, j * 128:(j + 1) * 128]
                if (kt + 1) * 128 > T:
                    col = kt * 128 + lax.broadcasted_iota(jnp.int32, (tq, 128), 1)
                    t = jnp.where(col < T, t, -jnp.inf)
                s_s[kt, 0:tq, :] = t
                mx = t if mx is None else jnp.maximum(mx, t)
                if G0 <= kt < G1:
                    cnt = (kt + 1 - G0) * npieces // (G1 - G0) - (kt - G0) * npieces // (G1 - G0)
                    for rr in range(cnt):
                        r = (tq * rr // cnt) // 8 * 8
                        conv_piece(*pieces.pop(0), t[r:r + 8, :])
        assert not pieces
        m = jnp.max(mx, axis=-1, keepdims=True)

        oc = _dot(z_s[...], wdm_s[...]) + x_s[b, pl.ds(r0, tq), :].astype(F32)

        rblocks = [(a, min(PR, tq - a)) for a in range(0, tq, PR)]
        ls = {}
        pblk = {}

        def exp_piece(c, a, n, gate):
            if gate is not None:
                s_s[0, pl.ds(spare_s, 8), :] = gate
            mm = m[a:a + n]
            ps = None
            tiles = []
            for j in range(TPC):
                p = jnp.exp2(s_s[c * TPC + j, a:a + n, :] - mm)
                ps = p if ps is None else ps + p
                tiles.append(p.astype(BF16))
            ls[a] = ps if a not in ls else ls[a] + ps
            pblk[c, a] = jnp.concatenate(tiles, axis=1)

        for c in range(AHEAD):
            for a, n in rblocks:
                exp_piece(c, a, n, None)
        acc = None
        for c in range(nkc):
            p = jnp.concatenate([pblk.pop((c, a)) for a, n in rblocks], axis=0)
            pv = _dot(p, v_s[c * KC:(c + 1) * KC, :])
            acc = pv if acc is None else acc + pv
            if c + AHEAD < nkc:
                for ib, (a, n) in enumerate(rblocks):
                    pos = ib * NL * tq // len(rblocks)
                    jj = pos // tq
                    r = (pos % tq) // 8 * 8
                    exp_piece(c + AHEAD, a, n, acc[r:r + 8, jj * 128:(jj + 1) * 128])
        l = jnp.sum(jnp.concatenate([ls[a] for a, n in rblocks], axis=0), axis=-1, keepdims=True)
        out = acc * (1.0 / l) + oc
        o_ref[0] = out.astype(o_ref.dtype)

    return pl.pallas_call(
        kernel,
        grid=(B, nq),
        in_specs=[pl.BlockSpec(memory_space=pl.ANY)] * 9,
        out_specs=pl.BlockSpec((1, tq, D), lambda b, i: (b, i, 0)),
        out_shape=jax.ShapeDtypeStruct((B, T, D), x.dtype),
        scratch_shapes=[
            pltpu.VMEM((B, T, D), BF16),
            pltpu.VMEM((D, D), BF16), pltpu.VMEM((D, D), BF16), pltpu.VMEM((D, D), BF16), pltpu.VMEM((D, D), BF16),
            pltpu.VMEM((D, 2 * D), BF16), pltpu.VMEM((K, D), BF16), pltpu.VMEM((D, D), BF16), pltpu.VMEM((2 * D, D), BF16),
            pltpu.SemaphoreType.DMA((9,)), pltpu.SemaphoreType.DMA((2 * B,)),
            pltpu.VMEM((D, D), BF16), pltpu.VMEM((D, D), BF16), pltpu.VMEM((D, D), BF16),
            pltpu.VMEM((K, 8, D), F32),
            pltpu.VMEM((TP, D), BF16), pltpu.VMEM((TP, D), BF16),
            pltpu.VMEM((NL, tq + 2 * HALO + 16, 128), F32), pltpu.VMEM((tq, D), F32), pltpu.VMEM((tq, D), BF16),
            pltpu.VMEM((TP // 128, tq + 16, 128), F32),
        ],
        compiler_params=pltpu.CompilerParams(
            dimension_semantics=("arbitrary", "arbitrary"),
            vmem_limit_bytes=100 * 1024 * 1024, flags=FLAGS,
        ),
    )(x, w_q, w_k, w_v, w_ao, w_up, dw, w_dn, w_merge)
```

```python
import math
import numpy as np
import jax
import jax.numpy as jnp
from jax import lax
import jax.experimental.pallas as pl
import jax.experimental.pallas.tpu as pltpu

H = 80
QC = 256
PC = 512
LB = 80
DLY = 3
ORD = 2
SUMT = 8
EXPT = 2
SPLIT = (45, 25, 10, 10)
QKM = 4
PVM = 1
SBW = (1, 1, 1, 2)
FLAGS = None
F32 = jnp.float32
BF16 = jnp.bfloat16
U32 = jnp.uint32


def _dot(a, b):
    return jnp.dot(a, b, preferred_element_type=F32)


def _dot_nt(a, b):
    return lax.dot_general(a, b, (((1,), (1,)), ((), ())), preferred_element_type=F32)


def _unpack(w):
    return pltpu.bitcast(w, BF16)


def _ln(x):
    m = jnp.mean(x, axis=-1, keepdims=True)
    xc = x - m
    v = jnp.mean(xc * xc, axis=-1, keepdims=True)
    return xc * lax.rsqrt(v + 1e-5)


def _gelu(x):
    c = math.sqrt(2.0 / math.pi)
    hx = 0.5 * x
    return hx + hx * jnp.tanh(x * (c + (c * 0.044715) * (x * x)))


def _lhs_combos(a11, a12, a21, a22):
    return (a11 + a22, a22 - a21, a11, a22, a11 - a12, a21 + a11, a12 + a22)


def _rhs_combos(b11, b12, b21, b22):
    return (b11 + b22, b11, b12 + b22, b21 + b11, b22, b12 - b11, b21 - b22)


def _quads(w):
    r, c = w.shape[0] // 2, w.shape[1] // 2
    return w[:r, :c], w[:r, c:], w[r:, :c], w[r:, c:]


def _seven(prod):
    n2 = prod(1)
    n4 = prod(3)
    c21 = n4 - n2
    n1 = prod(0)
    t11 = n1 - n4
    t22 = n1 - n2
    t11 = t11 + prod(6)
    n5 = prod(4)
    c11 = t11 - n5
    n3 = prod(2)
    c12 = n3 - n5
    c22 = (t22 - n3) + prod(5)
    return c11, c12, c21, c22


def _mix(*lists):
    keyed = [((n + 0.5) / len(l), k, n, w) for k, l in enumerate(lists) for n, w in enumerate(l)]
    return [e[3] for e in sorted(keyed, key=lambda e: e[:3])]


@jax.jit
def pallas_standalone__conformer_family_branchformer__speech_kernel(
    x, w_q, w_k, w_v, w_ao, w_up, dw, w_dn, w_merge,
):
    B, T, D = x.shape
    K = dw.shape[0]
    T2 = T // 2
    D2 = D // 2
    h = H
    nt = T2 // h
    TP = -(-T2 // PC) * PC
    NKT = TP // 128
    HALO = 16
    NL = D // 128
    assert (B * nt) % 2 == 0 and T2 % h == 0 and T2 % LB == 0 and TP >= T2 + HALO

    def kernel(x_hbm, wq_hbm, wk_hbm, wv_hbm, wao_hbm, wup_hbm, dw_hbm, wdn_hbm, wm_hbm, o_hbm,
               x_s, wq_s, wk_s, wv_s, wao_s, wup_s, dw_s, wdn_s, wm_s, wsem, xsem, osem,
               mc_s, uc_s, oc_s, dwb_s, xc_s, gi_s, o_s,
               gw_a, gw_b, z_a, z_b, s_a, s_b, zero_s):
        step = pl.program_id(0)
        nsteps = pl.num_programs(0)

        def x_copy(bb):
            return pltpu.make_async_copy(x_hbm.at[bb], x_s.at[bb], xsem.at[bb])

        def put_rhs(dst, k0, w):
            for i, c in enumerate(_rhs_combos(*_quads(w))):
                dst.bitcast(BF16)[i, k0:k0 + D2, :] = c.astype(BF16)

        @pl.when(step == 0)
        def _():
            top, bot = pl.ds(0, D), pl.ds(D, D)
            cp = [pltpu.make_async_copy(s, d, wsem.at[n]) for n, (s, d) in enumerate([
                (wao_hbm, wao_s), (wm_hbm.at[top], wm_s.at[top]), (wv_hbm, wv_s),
                (wq_hbm, wq_s), (wk_hbm, wk_s), (wdn_hbm, wdn_s), (wm_hbm.at[bot], wm_s.at[bot]),
                (dw_hbm, dw_s), (wup_hbm, wup_s)])]
            cp[0].start(); cp[1].start(); cp[2].start()
            zero_s[...] = jnp.zeros(zero_s.shape, U32)
            gw_a[...] = jnp.zeros(gw_a.shape, F32)
            gw_b[...] = jnp.zeros(gw_b.shape, F32)
            cp[0].wait(); cp[1].wait()
            cp[3].start(); cp[4].start()
            t = _dot(wao_s[...], wm_s[0:D, :]).astype(BF16)
            cp[2].wait()
            cp[5].start(); cp[6].start(); cp[7].start(); cp[8].start()
            put_rhs(oc_s, 0, _dot(wv_s[...], t))
            cp[3].wait(); cp[4].wait()
            x_copy(0).start()
            sc = float(D) ** -0.5 * math.log2(math.e)
            put_rhs(mc_s, 0, _dot_nt(wq_s[...], wk_s[...]) * sc)
            cp[5].wait(); cp[6].wait(); cp[7].wait(); cp[8].wait()
            put_rhs(oc_s, D2, _dot(wdn_s[...], wm_s[D:2 * D, :]))
            put_rhs(uc_s, 0, wup_s[:, 0:D].astype(F32))
            dwf = dw_s[...].astype(F32)
            for k in range(K):
                dwb_s[k] = jnp.broadcast_to(dwf[k:k + 1, :], (8, D))
            for bb in range(1, B):
                x_copy(bb).start()

        def put_x(bb, rows, top, bot):
            x11, x12, x21, x22 = top[:, :D2], top[:, D2:], bot[:, :D2], bot[:, D2:]
            for i, c in enumerate(_lhs_combos(x11, x12, x21, x22) + (x12, x21)):
                xc_s.bitcast(BF16)[bb, i, rows, :] = c.astype(BF16)

        for bb in range(B):
            @pl.when(step == (bb * nt) // 2)
            def _():
                x_copy(bb).wait()

                def body(r, carry):
                    r0 = pl.multiple_of(r * LB, 16)
                    top = _ln(x_s[bb, pl.ds(r0, LB), :].astype(F32))
                    bot = _ln(x_s[bb, pl.ds(T2 + r0, LB), :].astype(F32))
                    put_x(bb, pl.ds(r0, LB), top, bot)
                    return carry
                lax.fori_loop(0, T2 // LB, body, 0)
                mid = _ln(x_s[bb, T2 - HALO:T2 + HALO, :].astype(F32))
                put_x(bb, pl.ds(T2, HALO), mid[HALO:], jnp.zeros((HALO, D), F32))
                xc_s[bb, :, (T2 + HALO) // 2:, :] = jnp.zeros((9, (TP - T2 - HALO) // 2, D2), U32)
                head = _ln(x_s[bb, 0:HALO, :].astype(F32))
                xe = jnp.concatenate([head, mid], axis=0).astype(BF16)
                ge = _ln(_gelu(_dot(xe, wup_s[:, D:2 * D])))
                for j in range(NL):
                    gi_s[bb, 0, j, 0:HALO, :] = jnp.zeros((HALO, 128), F32)
                    gi_s[bb, 0, j, HALO:, :] = ge[0:HALO, j * 128:(j + 1) * 128]
                    gi_s[bb, 1, j, :, :] = ge[HALO:, j * 128:(j + 1) * 128]

        slot = step % 2
        spare8 = pl.multiple_of(8 * (2 * step // nt), 8)
        clock = [0]
        due = []

        def release(work, todo, val):
            for w in range(todo):
                rr = (h * w // todo) // 8 * 8
                due.append((clock[0] + DLY, work.pop(0)(val[rr:rr + 8, 0:128])))

        def mm(dot, lhs, w):
            bits = None
            due.sort(key=lambda e: e[0])
            while due and due[0][0] <= clock[0]:
                tok = pltpu.bitcast(due.pop(0)[1], U32)
                for a in range(0, tok.shape[0], 8):
                    bits = tok[a:a + 8] if bits is None else bits | tok[a:a + 8]
            if bits is not None:
                head = jnp.concatenate([w[0:8, 0:128] | (bits & zero_s[...]), w[0:8, 128:]], axis=1)
                w = jnp.concatenate([head, w[8:]], axis=0)
            r = dot(lhs, _unpack(w))
            due.append((clock[0] + ORD, r[0:8, 0:128]))
            clock[0] += 1
            return r

        class Tile:
            def __init__(self, t, gw, gw_prev, z, s):
                self.b = t // nt
                self.i = t % nt
                self.r0 = pl.multiple_of(self.i * h, 16)
                self.gw, self.gw_prev, self.z, self.s = gw, gw_prev, z, s
                self.lsum, self.lse, self.pc, self.zc = {}, {}, {}, {}

            def xc(self, i, off):
                rows = pl.ds(pl.multiple_of(self.i * (h // 2) + off // 2, 8), h // 2)
                return xc_s[self.b, i, rows, :]

            def proj(self, w_ref):
                return _seven(lambda i: mm(_dot, _unpack(self.xc(i, 0)), w_ref[i]))

            def proj_g(self):
                xg = jnp.concatenate([
                    jnp.concatenate([self.xc(2, HALO), self.xc(7, HALO)], axis=1),
                    jnp.concatenate([self.xc(8, HALO), self.xc(3, HALO)], axis=1)], axis=0)
                g = _ln(_gelu(_dot(_unpack(xg), wup_s[:, D:2 * D])))
                for hf in range(2):
                    for j in range(NL):
                        self.gw[hf, j, 0:2 * HALO, :] = jnp.where(
                            self.i == 0, gi_s[self.b, hf, j], self.gw_prev[hf, j, h:h + 2 * HALO, :])
                        self.gw[hf, j, 2 * HALO:h + 2 * HALO, :] = g[hf * h:(hf + 1) * h, j * 128:(j + 1) * 128]

            def proj_u(self):
                c11, c12, c21, c22 = self.proj(uc_s)
                for hf, (lo, hi) in enumerate(((c11, c12), (c21, c22))):
                    for n in range(2):
                        self.z[hf, n, 0:h, :] = _gelu(lo[:, n * 128:(n + 1) * 128])
                        self.z[hf, 2 + n, 0:h, :] = _gelu(hi[:, n * 128:(n + 1) * 128])

            def proj_q(self):
                q11, q12, q21, q22 = self.proj(mc_s)
                self.qc = [c.astype(BF16) for c in
                           (q11 + q22, q21 + q22, q11, q22, q11 + q12, q21 - q11, q12 - q22)]

            def conv_piece(self, hf, j, a, gate):
                self.gw[hf, j, pl.ds(h + 2 * HALO + spare8, 8), :] = gate
                acc = None
                for k in sorted(range(K), key=lambda k: (k % 8, k)):
                    w = dwb_s[k, :, j * 128:(j + 1) * 128]
                    t = self.gw[hf, j, a + k + 1:a + k + 17, :].reshape(2, 8, 128) * w[None]
                    acc = t if acc is None else acc + t
                z = acc.reshape(16, 128) * self.z[hf, j, a:a + 16, :]
                self.z[hf, j, a:a + 16, :] = z
                return z

            def z_piece(self, a, gate):
                self.z[0, 0, pl.ds(h + spare8, 8), :] = gate
                tiles = [_lhs_combos(*[self.z[hf, 2 * s + n, a:a + 16, :] for hf in range(2) for s in range(2)])
                         for n in range(2)]
                self.zc[a] = [jnp.concatenate([t[i] for t in tiles], axis=1) for i in range(7)]
                return tiles[1][6]

            def conv_pieces(self):
                work = []
                for a in range(0, h, 16):
                    work += [lambda g, hf=hf, j=j, a=a: self.conv_piece(hf, j, a, g)
                             for hf in range(2) for j in range(NL)]
                    work.append(lambda g, a=a: self.z_piece(a, g))
                return work

            def qk(self, work, margin):
                nchunk = TP // QC
                nslots = nchunk * 7 - margin
                total = len(work)
                mx = [None, None]
                cnt = [0]
                src = (0, 2, 1, 4, 3, 5, 6)

                for c in range(nchunk):
                    keys = pl.ds(c * QC // 2, QC // 2)

                    def prod(i):
                        r = mm(_dot_nt, self.qc[i], xc_s[self.b, src[i], keys, :])
                        n = cnt[0]
                        cnt[0] += 1
                        if n < nslots:
                            release(work, (n + 1) * total // nslots - n * total // nslots, r)
                        return r

                    def emit(hf, side, val):
                        for n in range(QC // 128):
                            kt = c * (QC // 128) + n
                            t = val[:, n * 128:(n + 1) * 128]
                            if (kt + 1) * 128 > T2:
                                col = kt * 128 + lax.broadcasted_iota(jnp.int32, (h, 128), 1)
                                t = jnp.where(col < T2, t, -jnp.inf)
                            self.s[hf, side, kt, 0:h, :] = t
                            mx[hf] = t if mx[hf] is None else jnp.maximum(mx[hf], t)

                    m2 = prod(1)
                    m4 = prod(3)
                    emit(1, 0, m2 - m4)
                    m1 = prod(0)
                    t11 = m1 - m4
                    t22 = m1 - m2
                    t11 = t11 + prod(6)
                    m5 = prod(4)
                    emit(0, 0, t11 - m5)
                    m3 = prod(2)
                    emit(0, 1, m5 - m3)
                    emit(1, 1, (t22 - m3) + prod(5))
                self.m = [jnp.max(v, axis=-1, keepdims=True) for v in mx]

            def gate_s(self, gate):
                self.s[0, 0, 0, pl.ds(h + spare8, 8), :] = gate

            def sum_piece(self, hf, a, tiles, last, gate):
                self.gate_s(gate)
                m = self.m[hf][a:a + 16]
                mb = jnp.broadcast_to(m, (16, 128))
                acc = self.lsum.get((hf, a))
                for side, kt in tiles:
                    e = jnp.exp2(self.s[hf, side, kt, a:a + 16, :] - mb)
                    acc = e if acc is None else acc + e
                self.lsum[hf, a] = acc
                if last:
                    l = jnp.sum(acc, axis=-1, keepdims=True)
                    acc = self.lse[hf, a] = jnp.broadcast_to(m + jnp.log2(l), (16, 128))
                return acc

            def sum_pieces(self):
                tiles = [(side, kt) for side in range(2) for kt in range(NKT) if kt * 128 < T2]
                work = []
                for a in range(0, h, 16):
                    work += [lambda g, hf=hf, a=a, n=n: self.sum_piece(hf, a, tiles[n:n + SUMT], n + SUMT >= len(tiles), g)
                             for hf in range(2) for n in range(0, len(tiles), SUMT)]
                    work += [lambda g, kt=kt, a=a: self.exp_piece(kt, a, g) for kt in range(0, PC // 128, EXPT)]
                return work

            def exp_piece(self, kt0, a, gate):
                self.gate_s(gate)
                tok = None
                for kt in range(kt0, kt0 + EXPT):
                    p = [jnp.exp2(self.s[hf, side, kt, a:a + 16, :] - self.lse[hf, a])
                         for hf in range(2) for side in range(2)]
                    cs = self.pc[kt, a] = _lhs_combos(*p)
                    t = cs[5] + cs[6]
                    tok = t if tok is None else tok + t
                return tok

            def exp_pieces(self, c):
                return [lambda g, kt=kt, a=a: self.exp_piece(kt, a, g)
                        for a in range(0, h, 16) for kt in range(c * PC // 128, (c + 1) * PC // 128, EXPT)]

            def pv(self, works):
                src = (0, 2, 6, 5, 3, 4, 1)
                acc = [None] * 7
                for c in range(TP // PC):
                    keys = pl.ds(c * PC // 2, PC // 2)
                    work = works[c]
                    total = len(work)
                    for n, i in enumerate((1, 3, 0, 6, 4, 2, 5)):
                        p = jnp.concatenate([
                            jnp.concatenate([self.pc[kt, a][i] for kt in range(c * PC // 128, (c + 1) * PC // 128)], axis=1)
                            for a in range(0, h, 16)], axis=0).astype(BF16)
                        r = mm(_dot, p, xc_s[self.b, src[i], keys, :])
                        acc[i] = r if acc[i] is None else acc[i] + r
                        if n < 7 - PVM:
                            release(work, (n + 1) * total // (7 - PVM) - n * total // (7 - PVM), acc[i])
                n1, n2, n3, n4, n5, n6, n7 = acc
                self.oc = _lhs_combos(n1 - n4 - n5 - n7, n3 - n5, n4 - n2, n1 - n2 - n3 - n6)

            def out(self, dst):
                zc = [jnp.concatenate([self.zc[a][i] for a in range(0, h, 16)], axis=0) for i in range(7)]
                c11, c12, c21, c22 = _seven(
                    lambda i: mm(_dot, jnp.concatenate([self.oc[i], zc[i]], axis=1).astype(BF16), oc_s[i]))
                for hf, (lo, hi) in enumerate(((c11, c12), (c21, c22))):
                    res = x_s[self.b, pl.ds(pl.multiple_of(hf * T2 + self.r0, 16), h), :].astype(F32)
                    o_s[slot, dst, hf] = (jnp.concatenate([lo, hi], axis=1) + res).astype(o_s.dtype)

            def out_copy(self, sl, dst):
                return pltpu.make_async_copy(
                    o_s.at[sl, dst], o_hbm.at[self.b, :, pl.ds(self.r0, h), :], osem.at[sl, dst])

        ta = Tile(2 * step, gw_a, gw_b, z_a, s_a)
        tb = Tile(2 * step + 1, gw_b, gw_a, z_b, s_b)

        @pl.when(step >= 2)
        def _():
            ta.out_copy(slot, 0).wait()
            tb.out_copy(slot, 1).wait()

        npv = TP // PC
        conv = ta.conv_pieces() + tb.conv_pieces()
        assert sum(SPLIT) == len(conv)
        cw = [conv[sum(SPLIT[:n]):sum(SPLIT[:n + 1])] for n in range(4)]

        def part(l, c, n):
            return l[c * len(l) // n:(c + 1) * len(l) // n] if c < n else []

        ta.proj_g(); ta.proj_u(); ta.proj_q()
        tb.proj_g(); tb.proj_u(); tb.proj_q()
        ta.qk(cw[0], 0)
        tb.qk(_mix(cw[1], ta.sum_pieces()), QKM)
        sb = tb.sum_pieces()
        cut = [len(sb) * n // sum(SBW) for n in np.cumsum((0,) + SBW)]
        ta.pv([_mix(ta.exp_pieces(c + 1) if c + 1 < npv else [],
                    sb[cut[c]:cut[c + 1]], part(cw[2], c, npv)) for c in range(npv)])
        tb.pv([_mix(tb.exp_pieces(c + 1) if c + 1 < npv else [], part(cw[3], npv - 1 - c, 1)) for c in range(npv)])
        ta.out(0)
        tb.out(1)
        ta.out_copy(slot, 0).start()
        tb.out_copy(slot, 1).start()

        @pl.when(step == nsteps - 1)
        def _():
            ta.out_copy(slot, 0).wait()
            tb.out_copy(slot, 1).wait()
            ta.out_copy(1 - slot, 0).wait()
            tb.out_copy(1 - slot, 1).wait()

    gw_shape = (2, NL, h + 2 * HALO + 16, 128)
    z_shape = (2, NL, h + 16, 128)
    s_shape = (2, 2, NKT, h + 16, 128)
    out = pl.pallas_call(
        kernel,
        grid=(B * nt // 2,),
        in_specs=[pl.BlockSpec(memory_space=pl.ANY)] * 9,
        out_specs=pl.BlockSpec(memory_space=pl.ANY),
        out_shape=jax.ShapeDtypeStruct((B, 2, T2, D), x.dtype),
        scratch_shapes=[
            pltpu.VMEM((B, T, D), BF16),
            pltpu.VMEM((D, D), BF16), pltpu.VMEM((D, D), BF16), pltpu.VMEM((D, D), BF16), pltpu.VMEM((D, D), BF16),
            pltpu.VMEM((D, 2 * D), BF16), pltpu.VMEM((K, D), BF16), pltpu.VMEM((D, D), BF16), pltpu.VMEM((2 * D, D), BF16),
            pltpu.SemaphoreType.DMA((9,)), pltpu.SemaphoreType.DMA((B,)), pltpu.SemaphoreType.DMA((2, 2)),
            pltpu.VMEM((7, D2 // 2, D2), U32), pltpu.VMEM((7, D2 // 2, D2), U32), pltpu.VMEM((7, D2, D2), U32),
            pltpu.VMEM((K, 8, D), F32),
            pltpu.VMEM((B, 9, TP // 2, D2), U32),
            pltpu.VMEM((B, 2, NL, 2 * HALO, 128), F32),
            pltpu.VMEM((2, 2, 2, h, D), x.dtype),
            pltpu.VMEM(gw_shape, F32), pltpu.VMEM(gw_shape, F32),
            pltpu.VMEM(z_shape, F32), pltpu.VMEM(z_shape, F32),
            pltpu.VMEM(s_shape, F32), pltpu.VMEM(s_shape, F32),
            pltpu.VMEM((8, 128), U32),
        ],
        compiler_params=pltpu.CompilerParams(
            dimension_semantics=("arbitrary",),
            vmem_limit_bytes=100 * 1024 * 1024, flags=FLAGS,
        ),
    )(x, w_q, w_k, w_v, w_ao, w_up, dw, w_dn, w_merge)
    return out.reshape(B, T, D)
```

```python
import math
import numpy as np
import jax
import jax.numpy as jnp
from jax import lax
import jax.experimental.pallas as pl
import jax.experimental.pallas.tpu as pltpu

H = 80
QC = 256
PC = 512
LB = 80
AHEAD = 2
DLY = 6
ORD = 2
SUMT = 8
EXPT = 2
SPLIT = (55, 15, 5, 15)
QKM = 4
PVM = 1
SBW = (1, 1, 1, 2)
FLAGS = None
F32 = jnp.float32
BF16 = jnp.bfloat16
U32 = jnp.uint32


def _dot(a, b):
    return jnp.dot(a, b, preferred_element_type=F32)


def _dot_nt(a, b):
    return lax.dot_general(a, b, (((1,), (1,)), ((), ())), preferred_element_type=F32)


def _unpack(w):
    return pltpu.bitcast(w, BF16)


def _ln(x):
    m = jnp.mean(x, axis=-1, keepdims=True)
    xc = x - m
    v = jnp.mean(xc * xc, axis=-1, keepdims=True)
    return xc * lax.rsqrt(v + 1e-5)


def _gelu(x):
    c = math.sqrt(2.0 / math.pi)
    hx = 0.5 * x
    return hx + hx * jnp.tanh(x * (c + (c * 0.044715) * (x * x)))


def _lhs_combos(a11, a12, a21, a22):
    return (a11 + a22, a22 - a21, a11, a22, a11 - a12, a21 + a11, a12 + a22)


def _rhs_combos(b11, b12, b21, b22):
    return (b11 + b22, b11, b12 + b22, b21 + b11, b22, b12 - b11, b21 - b22)


def _quads(w):
    r, c = w.shape[0] // 2, w.shape[1] // 2
    return w[:r, :c], w[:r, c:], w[r:, :c], w[r:, c:]


def _seven(prod):
    n2 = prod(1)
    n4 = prod(3)
    c21 = n4 - n2
    n1 = prod(0)
    t11 = n1 - n4
    t22 = n1 - n2
    t11 = t11 + prod(6)
    n5 = prod(4)
    c11 = t11 - n5
    n3 = prod(2)
    c12 = n3 - n5
    c22 = (t22 - n3) + prod(5)
    return c11, c12, c21, c22


def _mix(*lists):
    keyed = [((n + 0.5) / len(l), k, n, w) for k, l in enumerate(lists) for n, w in enumerate(l)]
    return [e[3] for e in sorted(keyed, key=lambda e: e[:3])]


@jax.jit
def pallas_standalone__conformer_family_branchformer__speech_kernel(
    x, w_q, w_k, w_v, w_ao, w_up, dw, w_dn, w_merge,
):
    B, T, D = x.shape
    K = dw.shape[0]
    T2 = T // 2
    D2 = D // 2
    h = H
    nt = T2 // h
    TP = -(-T2 // PC) * PC
    NKT = TP // 128
    HALO = 16
    NL = D // 128
    assert B == 2 and (B * nt) % 2 == 0 and T2 % h == 0 and T2 % LB == 0 and TP >= T2 + HALO

    def kernel(x_hbm, wq_hbm, wk_hbm, wv_hbm, wao_hbm, wup_hbm, dw_hbm, wdn_hbm, wm_hbm, o_hbm,
               x_s, wq_s, wk_s, wv_s, wao_s, wup_s, dw_s, wdn_s, wm_s, wsem, xsem, osem,
               mc_s, uc_s, oc_s, dwb_s, xc_s, gi_s, o_s,
               gw_a, gw_b, z_a, z_b, s_a, s_b, zero_s, st_s, fsem, t_s):
        step = pl.program_id(0)
        nsteps = pl.num_programs(0)

        def ln_rows(top, bot):
            parts = []
            for v in (top, bot):
                w = pltpu.bitcast(v, U32)
                parts.append([_ln(pltpu.bitcast(u, F32)) for u in (w << 16, w & np.uint32(0xFFFF0000))])
            sets = []
            for par in range(2):
                t, b = parts[0][par], parts[1][par]
                x11, x12, x21, x22 = t[:, :D2], t[:, D2:], b[:, :D2], b[:, D2:]
                sets.append(_lhs_combos(x11, x12, x21, x22) + (x12, x21))
            return [pltpu.pack_elementwise([e, o], packed_dtype=BF16) for e, o in zip(*sets)]

        def edges(bb):
            over = x_s[bb, 1, 0:HALO, :]
            for i, c in enumerate(ln_rows(over, jnp.zeros((HALO, D), BF16))):
                xc_s[bb, i, T2 // 2:(T2 + HALO) // 2, :] = c
            xc_s[bb, :, (T2 + HALO) // 2:, :] = jnp.zeros((9, (TP - T2 - HALO) // 2, D2), U32)
            xe = jnp.concatenate([x_s[bb, 0, 0:HALO, :], x_s[bb, 0, T2 - HALO:T2, :], over], axis=0)
            ge = _ln(_gelu(_dot(_ln(xe.astype(F32)).astype(BF16), wup_s[:, D:2 * D])))
            for j in range(NL):
                gi_s[bb, 0, j, 0:HALO, :] = jnp.zeros((HALO, 128), F32)
                gi_s[bb, 0, j, HALO:, :] = ge[0:HALO, j * 128:(j + 1) * 128]
                gi_s[bb, 1, j, :, :] = ge[HALO:, j * 128:(j + 1) * 128]

        def x_copy(bb, r0, r1, n):
            rows = (bb, slice(None), pl.ds(r0, r1 - r0))
            return pltpu.make_async_copy(x_hbm.at[rows], x_s.at[rows], xsem.at[n])

        @pl.when(step == 0)
        def _():
            top, bot = pl.ds(0, D), pl.ds(D, D)
            cp = [pltpu.make_async_copy(s, d, wsem.at[n]) for n, (s, d) in enumerate([
                (wao_hbm, wao_s), (wm_hbm.at[top], wm_s.at[top]), (wv_hbm, wv_s),
                (wq_hbm, wq_s), (wk_hbm, wk_s), (wdn_hbm, wdn_s), (wm_hbm.at[bot], wm_s.at[bot]),
                (dw_hbm, dw_s), (wup_hbm, wup_s)])]
            cuts = [T2 // 16 * n // 4 * 16 for n in range(5)]
            xp = [x_copy(0, cuts[n], cuts[n + 1], n) for n in range(4)]
            stages = [[cp[0], cp[1], xp[0]], [cp[2], xp[1]], [cp[3], cp[4], xp[2]], [cp[5], cp[6], xp[3]],
                      [cp[7], cp[8]]]
            started = [0]

            def arrive(n):
                while started[0] < min(n + 1 + AHEAD, len(stages)):
                    for c in stages[started[0]]:
                        c.start()
                    started[0] += 1
                for c in stages[n]:
                    c.wait()

            def stage(n, dot, lhs_ref, rhs, put):
                nsub = 4
                sub = [cuts[n] + (cuts[n + 1] - cuts[n]) // 16 * k // nsub * 16 for k in range(nsub + 1)]
                wr = D2 // nsub
                for k in range(nsub):
                    lhs = jnp.concatenate([lhs_ref[k * wr:(k + 1) * wr, :],
                                           lhs_ref[D2 + k * wr:D2 + (k + 1) * wr, :]], axis=0)
                    put(k * wr, wr, dot(lhs, rhs()))
                    r0, r1 = sub[k], sub[k + 1]
                    for i, c in enumerate(ln_rows(x_s[0, 0, r0:r1, :], x_s[0, 1, r0:r1, :])):
                        xc_s[0, i, r0 // 2:r1 // 2, :] = c

            def put_plain(r, n, w):
                t_s[r:r + n, :] = w[:n].astype(BF16)
                t_s[D2 + r:D2 + r + n, :] = w[n:].astype(BF16)

            def put_rhs(dst, k0, scale=None):
                def put(r, n, w):
                    if scale is not None:
                        w = w * scale
                    for i, c in enumerate(_rhs_combos(*_quads(w))):
                        dst.bitcast(BF16)[i, k0 + r:k0 + r + n, :] = c.astype(BF16)
                return put

            arrive(0)
            zero_s[...] = jnp.zeros(zero_s.shape, U32)
            gw_b[:, :, h:h + 2 * HALO, :] = jnp.zeros((2, NL, 2 * HALO, 128), F32)
            stage(0, _dot, wao_s, lambda: wm_s[0:D, :], put_plain)
            arrive(1)
            stage(1, _dot, wv_s, lambda: t_s[...], put_rhs(oc_s, 0))
            arrive(2)
            stage(2, _dot_nt, wq_s, lambda: wk_s[...], put_rhs(mc_s, 0, float(D) ** -0.5 * math.log2(math.e)))
            arrive(3)
            stage(3, _dot, wdn_s, lambda: wm_s[D:2 * D, :], put_rhs(oc_s, D2))
            arrive(4)
            x_copy(1, 0, T2, 4).start()
            for r in range(0, D2, 64):
                halves = []
                for r0 in (r, D2 + r):
                    w = pltpu.bitcast(wup_s[r0:r0 + 64, 0:D], U32)
                    halves.append([pltpu.bitcast(u, F32) for u in (w << 16, w & np.uint32(0xFFFF0000))])
                sets = [_rhs_combos(t[:, :D2], t[:, D2:], b[:, :D2], b[:, D2:]) for t, b in zip(*halves)]
                for i, (e, o) in enumerate(zip(*sets)):
                    uc_s[i, r // 2:r // 2 + 32, :] = pltpu.pack_elementwise([e, o], packed_dtype=BF16)
            dwf = dw_s[...].astype(F32)
            for k in range(K):
                dwb_s[k] = jnp.broadcast_to(dwf[k:k + 1, :], (8, D))
            edges(0)

        first = nt // 2
        nfill = first - 2
        fill_rows = -(-(T2 // 16) // nfill) * 16
        last_rows = T2 - (nfill - 1) * fill_rows

        def fill_copy(s, rows):
            dst = pl.ds(pl.multiple_of((s - 1) * (fill_rows // 2), 8), rows // 2)
            return pltpu.make_async_copy(st_s.at[s % 2, :, pl.ds(0, rows // 2)], xc_s.at[1, :, dst], fsem.at[s % 2])

        @pl.when(step == 1)
        def _():
            x_copy(1, 0, T2, 4).wait()

        @pl.when((step >= 3) & (step < first))
        def _():
            fill_copy(step - 2, fill_rows).wait()

        @pl.when(step == first)
        def _():
            fill_copy(step - 2, last_rows).wait()
            edges(1)

        slot = step % 2
        spare8 = pl.multiple_of(8 * (2 * step // nt), 8)
        clock = [0]
        due = []

        def release(work, todo, val):
            for w in range(todo):
                rr = (h * w // todo) // 8 * 8
                due.append((clock[0] + DLY, work.pop(0)(val[rr:rr + 8, 0:128])))

        def mm(dot, lhs, w):
            bits = None
            due.sort(key=lambda e: e[0])
            while due and due[0][0] <= clock[0]:
                tok = pltpu.bitcast(due.pop(0)[1], U32)
                for a in range(0, tok.shape[0], 8):
                    bits = tok[a:a + 8] if bits is None else bits | tok[a:a + 8]
            if bits is not None:
                head = jnp.concatenate([w[0:8, 0:128] | (bits & zero_s[...]), w[0:8, 128:]], axis=1)
                w = jnp.concatenate([head, w[8:]], axis=0)
            r = dot(lhs, _unpack(w))
            due.append((clock[0] + ORD, r[0:8, 0:128]))
            clock[0] += 1
            return r

        class Tile:
            def __init__(self, t, gw, gw_prev, z, s):
                self.b = t // nt
                self.i = t % nt
                self.r0 = pl.multiple_of(self.i * h, 16)
                self.gw, self.gw_prev, self.z, self.s = gw, gw_prev, z, s
                self.lsum, self.lse, self.pc, self.zc = {}, {}, {}, {}

            def xc(self, i, off):
                rows = pl.ds(pl.multiple_of(self.i * (h // 2) + off // 2, 8), h // 2)
                return xc_s[self.b, i, rows, :]

            def proj(self, w_ref):
                return _seven(lambda i: mm(_dot, _unpack(self.xc(i, 0)), w_ref[i]))

            def proj_g(self):
                xg = jnp.concatenate([
                    jnp.concatenate([self.xc(2, HALO), self.xc(7, HALO)], axis=1),
                    jnp.concatenate([self.xc(8, HALO), self.xc(3, HALO)], axis=1)], axis=0)
                g = _ln(_gelu(_dot(_unpack(xg), wup_s[:, D:2 * D])))
                for hf in range(2):
                    for j in range(NL):
                        self.gw[hf, j, 0:2 * HALO, :] = jnp.where(
                            self.i == 0, gi_s[self.b, hf, j], self.gw_prev[hf, j, h:h + 2 * HALO, :])
                        self.gw[hf, j, 2 * HALO:h + 2 * HALO, :] = g[hf * h:(hf + 1) * h, j * 128:(j + 1) * 128]

            def proj_u(self):
                c11, c12, c21, c22 = self.proj(uc_s)
                for hf, (lo, hi) in enumerate(((c11, c12), (c21, c22))):
                    for n in range(2):
                        self.z[hf, n, 0:h, :] = _gelu(lo[:, n * 128:(n + 1) * 128])
                        self.z[hf, 2 + n, 0:h, :] = _gelu(hi[:, n * 128:(n + 1) * 128])

            def proj_q(self):
                q11, q12, q21, q22 = self.proj(mc_s)
                self.qc = [c.astype(BF16) for c in
                           (q11 + q22, q21 + q22, q11, q22, q11 + q12, q21 - q11, q12 - q22)]

            def conv_piece(self, hf, j, a, gate):
                self.gw[hf, j, pl.ds(h + 2 * HALO + spare8, 8), :] = gate
                acc = None
                for k in sorted(range(K), key=lambda k: (k % 8, k)):
                    w = dwb_s[k, :, j * 128:(j + 1) * 128]
                    t = self.gw[hf, j, a + k + 1:a + k + 17, :].reshape(2, 8, 128) * w[None]
                    acc = t if acc is None else acc + t
                z = acc.reshape(16, 128) * self.z[hf, j, a:a + 16, :]
                self.z[hf, j, a:a + 16, :] = z
                return z

            def z_piece(self, a, gate):
                self.z[0, 0, pl.ds(h + spare8, 8), :] = gate
                tiles = [_lhs_combos(*[self.z[hf, 2 * s + n, a:a + 16, :] for hf in range(2) for s in range(2)])
                         for n in range(2)]
                self.zc[a] = [jnp.concatenate([t[i] for t in tiles], axis=1) for i in range(7)]
                return tiles[1][6]

            def conv_pieces(self):
                work = []
                for a in range(0, h, 16):
                    work += [lambda g, hf=hf, j=j, a=a: self.conv_piece(hf, j, a, g)
                             for hf in range(2) for j in range(NL)]
                    work.append(lambda g, a=a: self.z_piece(a, g))
                return work

            def qk(self, work, margin):
                nchunk = TP // QC
                nslots = nchunk * 7 - margin
                total = len(work)
                mx = [None, None]
                cnt = [0]
                src = (0, 2, 1, 4, 3, 5, 6)

                for c in range(nchunk):
                    keys = pl.ds(c * QC // 2, QC // 2)

                    def prod(i):
                        r = mm(_dot_nt, self.qc[i], xc_s[self.b, src[i], keys, :])
                        n = cnt[0]
                        cnt[0] += 1
                        if n < nslots:
                            release(work, (n + 1) * total // nslots - n * total // nslots, r)
                        return r

                    def emit(hf, side, val):
                        for n in range(QC // 128):
                            kt = c * (QC // 128) + n
                            t = val[:, n * 128:(n + 1) * 128]
                            if (kt + 1) * 128 > T2:
                                col = kt * 128 + lax.broadcasted_iota(jnp.int32, (h, 128), 1)
                                t = jnp.where(col < T2, t, -jnp.inf)
                            self.s[hf, side, kt, 0:h, :] = t
                            mx[hf] = t if mx[hf] is None else jnp.maximum(mx[hf], t)

                    m2 = prod(1)
                    m4 = prod(3)
                    emit(1, 0, m2 - m4)
                    m1 = prod(0)
                    t11 = m1 - m4
                    t22 = m1 - m2
                    t11 = t11 + prod(6)
                    m5 = prod(4)
                    emit(0, 0, t11 - m5)
                    m3 = prod(2)
                    emit(0, 1, m5 - m3)
                    emit(1, 1, (t22 - m3) + prod(5))
                self.m = [jnp.max(v, axis=-1, keepdims=True) for v in mx]

            def gate_s(self, gate):
                self.s[0, 0, 0, pl.ds(h + spare8, 8), :] = gate

            def sum_piece(self, hf, a, tiles, last, gate):
                self.gate_s(gate)
                m = self.m[hf][a:a + 16]
                mb = jnp.broadcast_to(m, (16, 128))
                acc = self.lsum.get((hf, a))
                for side, kt in tiles:
                    e = jnp.exp2(self.s[hf, side, kt, a:a + 16, :] - mb)
                    acc = e if acc is None else acc + e
                self.lsum[hf, a] = acc
                if last:
                    l = jnp.sum(acc, axis=-1, keepdims=True)
                    acc = self.lse[hf, a] = jnp.broadcast_to(m + jnp.log2(l), (16, 128))
                return acc

            def sum_pieces(self):
                tiles = [(side, kt) for side in range(2) for kt in range(NKT) if kt * 128 < T2]
                work = []
                for a in range(0, h, 16):
                    work += [lambda g, hf=hf, a=a, n=n: self.sum_piece(hf, a, tiles[n:n + SUMT], n + SUMT >= len(tiles), g)
                             for hf in range(2) for n in range(0, len(tiles), SUMT)]
                    work += [lambda g, kt=kt, a=a: self.exp_piece(kt, a, g) for kt in range(0, PC // 128, EXPT)]
                return work

            def exp_piece(self, kt0, a, gate):
                self.gate_s(gate)
                tok = None
                for kt in range(kt0, kt0 + EXPT):
                    p = [jnp.exp2(self.s[hf, side, kt, a:a + 16, :] - self.lse[hf, a])
                         for hf in range(2) for side in range(2)]
                    cs = self.pc[kt, a] = _lhs_combos(*p)
                    t = cs[5] + cs[6]
                    tok = t if tok is None else tok + t
                return tok

            def exp_pieces(self, c):
                return [lambda g, kt=kt, a=a: self.exp_piece(kt, a, g)
                        for a in range(0, h, 16) for kt in range(c * PC // 128, (c + 1) * PC // 128, EXPT)]

            def pv(self, works):
                src = (0, 2, 6, 5, 3, 4, 1)
                acc = [None] * 7
                for c in range(TP // PC):
                    keys = pl.ds(c * PC // 2, PC // 2)
                    work = works[c]
                    total = len(work)
                    for n, i in enumerate((1, 3, 0, 6, 4, 2, 5)):
                        p = jnp.concatenate([
                            jnp.concatenate([self.pc[kt, a][i] for kt in range(c * PC // 128, (c + 1) * PC // 128)], axis=1)
                            for a in range(0, h, 16)], axis=0).astype(BF16)
                        r = mm(_dot, p, xc_s[self.b, src[i], keys, :])
                        acc[i] = r if acc[i] is None else acc[i] + r
                        if n < 7 - PVM:
                            release(work, (n + 1) * total // (7 - PVM) - n * total // (7 - PVM), acc[i])
                n1, n2, n3, n4, n5, n6, n7 = acc
                self.oc = _lhs_combos(n1 - n4 - n5 - n7, n3 - n5, n4 - n2, n1 - n2 - n3 - n6)

            def out(self, dst):
                zc = [jnp.concatenate([self.zc[a][i] for a in range(0, h, 16)], axis=0) for i in range(7)]
                c11, c12, c21, c22 = _seven(
                    lambda i: mm(_dot, jnp.concatenate([self.oc[i], zc[i]], axis=1).astype(BF16), oc_s[i]))
                for hf, (lo, hi) in enumerate(((c11, c12), (c21, c22))):
                    res = x_s[self.b, hf, pl.ds(self.r0, h), :].astype(F32)
                    o_s[slot, dst, hf] = (jnp.concatenate([lo, hi], axis=1) + res).astype(o_s.dtype)

            def out_copy(self, sl, dst):
                return pltpu.make_async_copy(
                    o_s.at[sl, dst], o_hbm.at[self.b, :, pl.ds(self.r0, h), :], osem.at[sl, dst])

        ta = Tile(2 * step, gw_a, gw_b, z_a, s_a)
        tb = Tile(2 * step + 1, gw_b, gw_a, z_b, s_b)

        @pl.when(step >= 2)
        def _():
            ta.out_copy(slot, 0).wait()
            tb.out_copy(slot, 1).wait()

        npv = TP // PC
        conv = ta.conv_pieces() + tb.conv_pieces()
        assert sum(SPLIT) == len(conv)
        cw = [conv[sum(SPLIT[:n]):sum(SPLIT[:n + 1])] for n in range(4)]

        def part(l, c, n):
            return l[c * len(l) // n:(c + 1) * len(l) // n] if c < n else []

        ta.proj_g(); ta.proj_u(); ta.proj_q()
        tb.proj_g(); tb.proj_u(); tb.proj_q()
        def fill_piece(n, gate):
            r = jnp.clip((step - 1) * fill_rows + n * 16, 0, T2 - 16)
            rows = pl.ds(pl.multiple_of(r, 16), 16)
            bb = jnp.minimum(step, 1)
            hold = pltpu.bitcast(gate, U32) & zero_s[...]
            top, bot = [_unpack(pltpu.bitcast(x_s[bb, hf, rows, :], U32) | jnp.concatenate([hold] * NL, axis=1))
                        for hf in range(2)]
            cs = ln_rows(top, bot)
            for i, c in enumerate(cs):
                st_s[slot, i, n * 8:n * 8 + 8, :] = c
            return cs[0][:, 0:128]

        fills = [lambda g, n=n: fill_piece(n, g) for n in range(fill_rows // 16)]
        ta.qk(cw[0], 0)
        tb.qk(_mix(cw[1], ta.sum_pieces()), QKM)
        sb = tb.sum_pieces()
        cut = [len(sb) * n // sum(SBW) for n in np.cumsum((0,) + SBW)]
        ta.pv([_mix(ta.exp_pieces(c + 1) if c + 1 < npv else [],
                    sb[cut[c]:cut[c + 1]], part(cw[2], c, npv)) for c in range(npv)])
        tb.pv([_mix(tb.exp_pieces(c + 1) if c + 1 < npv else [], part(cw[3], npv - 1 - c, 1),
                    part(fills, c, npv - 1)) for c in range(npv)])
        ta.out(0)
        tb.out(1)
        ta.out_copy(slot, 0).start()
        tb.out_copy(slot, 1).start()

        @pl.when((step >= 1) & (step < nfill))
        def _():
            fill_copy(step, fill_rows).start()

        @pl.when(step == nfill)
        def _():
            fill_copy(step, last_rows).start()

        @pl.when(step == nsteps - 1)
        def _():
            ta.out_copy(slot, 0).wait()
            tb.out_copy(slot, 1).wait()
            ta.out_copy(1 - slot, 0).wait()
            tb.out_copy(1 - slot, 1).wait()

    gw_shape = (2, NL, h + 2 * HALO + 16, 128)
    z_shape = (2, NL, h + 16, 128)
    s_shape = (2, 2, NKT, h + 16, 128)
    out = pl.pallas_call(
        kernel,
        grid=(B * nt // 2,),
        in_specs=[pl.BlockSpec(memory_space=pl.ANY)] * 9,
        out_specs=pl.BlockSpec(memory_space=pl.ANY),
        out_shape=jax.ShapeDtypeStruct((B, 2, T2, D), x.dtype),
        scratch_shapes=[
            pltpu.VMEM((B, 2, T2, D), BF16),
            pltpu.VMEM((D, D), BF16), pltpu.VMEM((D, D), BF16), pltpu.VMEM((D, D), BF16), pltpu.VMEM((D, D), BF16),
            pltpu.VMEM((D, 2 * D), BF16), pltpu.VMEM((K, D), BF16), pltpu.VMEM((D, D), BF16), pltpu.VMEM((2 * D, D), BF16),
            pltpu.SemaphoreType.DMA((9,)), pltpu.SemaphoreType.DMA((5,)), pltpu.SemaphoreType.DMA((2, 2)),
            pltpu.VMEM((7, D2 // 2, D2), U32), pltpu.VMEM((7, D2 // 2, D2), U32), pltpu.VMEM((7, D2, D2), U32),
            pltpu.VMEM((K, 8, D), F32),
            pltpu.VMEM((B, 9, TP // 2, D2), U32),
            pltpu.VMEM((B, 2, NL, 2 * HALO, 128), F32),
            pltpu.VMEM((2, 2, 2, h, D), x.dtype),
            pltpu.VMEM(gw_shape, F32), pltpu.VMEM(gw_shape, F32),
            pltpu.VMEM(z_shape, F32), pltpu.VMEM(z_shape, F32),
            pltpu.VMEM(s_shape, F32), pltpu.VMEM(s_shape, F32),
            pltpu.VMEM((8, 128), U32),
            pltpu.VMEM((2, 9, -(-(T2 // 16) // (nt // 2 - 2)) * 8, D2), U32), pltpu.SemaphoreType.DMA((2,)),
            pltpu.VMEM((D, D), BF16),
        ],
        compiler_params=pltpu.CompilerParams(
            dimension_semantics=("arbitrary",),
            vmem_limit_bytes=100 * 1024 * 1024, flags=FLAGS,
        ),
    )(x.reshape(B, 2, T2, D), w_q, w_k, w_v, w_ao, w_up, dw, w_dn, w_merge)
    return out.reshape(B, T, D)
```

```python
import math
import numpy as np
import jax
import jax.numpy as jnp
from jax import lax
import jax.experimental.pallas as pl
import jax.experimental.pallas.tpu as pltpu

H = 80
QC = 256
PC = 512
LB = 80
AHEAD = 2
CR = 16
DLY = 6
ORD = 3
SUMT = 8
EXPT = 2
SPLIT = (55, 15, 5, 15)
QKM = 4
PVM = 1
SBW = (1, 1, 1, 2)
NOBC = True
LATE = False
QORD = 1
FLAGS = None
F32 = jnp.float32
BF16 = jnp.bfloat16
U32 = jnp.uint32


def _dot(a, b):
    return jnp.dot(a, b, preferred_element_type=F32)


def _dot_nt(a, b):
    return lax.dot_general(a, b, (((1,), (1,)), ((), ())), preferred_element_type=F32)


def _unpack(w):
    return pltpu.bitcast(w, BF16)


def _ln(x):
    m = jnp.mean(x, axis=-1, keepdims=True)
    xc = x - m
    v = jnp.mean(xc * xc, axis=-1, keepdims=True)
    return xc * lax.rsqrt(v + 1e-5)


def _gelu(x):
    c = math.sqrt(2.0 / math.pi)
    hx = 0.5 * x
    return hx + hx * jnp.tanh(x * (c + (c * 0.044715) * (x * x)))


def _lhs_combos(a11, a12, a21, a22):
    return (a11 + a22, a22 - a21, a11, a22, a11 - a12, a21 + a11, a12 + a22)


def _rhs_combos(b11, b12, b21, b22):
    return (b11 + b22, b11, b12 + b22, b21 + b11, b22, b12 - b11, b21 - b22)


def _quads(w):
    r, c = w.shape[0] // 2, w.shape[1] // 2
    return w[:r, :c], w[:r, c:], w[r:, :c], w[r:, c:]


def _seven(prod):
    n2 = prod(1)
    n4 = prod(3)
    c21 = n4 - n2
    n1 = prod(0)
    t11 = n1 - n4
    t22 = n1 - n2
    t11 = t11 + prod(6)
    n5 = prod(4)
    c11 = t11 - n5
    n3 = prod(2)
    c12 = n3 - n5
    c22 = (t22 - n3) + prod(5)
    return c11, c12, c21, c22


def _mix(*lists):
    keyed = [((n + 0.5) / len(l), k, n, w) for k, l in enumerate(lists) for n, w in enumerate(l)]
    return [e[3] for e in sorted(keyed, key=lambda e: e[:3])]


@jax.jit
def pallas_standalone__conformer_family_branchformer__speech_kernel(
    x, w_q, w_k, w_v, w_ao, w_up, dw, w_dn, w_merge,
):
    B, T, D = x.shape
    K = dw.shape[0]
    T2 = T // 2
    D2 = D // 2
    h = H
    nt = T2 // h
    TP = -(-T2 // PC) * PC
    NKT = TP // 128
    HALO = 16
    NL = D // 128
    assert B == 2 and (B * nt) % 2 == 0 and T2 % h == 0 and T2 % LB == 0 and TP >= T2 + HALO

    def kernel(x_hbm, wq_hbm, wk_hbm, wv_hbm, wao_hbm, wup_hbm, dw_hbm, wdn_hbm, wm_hbm, o_hbm,
               x_s, wq_s, wk_s, wv_s, wao_s, wup_s, dw_s, wdn_s, wm_s, wsem, xsem, osem,
               mc_s, uc_s, oc_s, dwb_s, xc_s, gi_s, o_s,
               gw_a, gw_b, z_a, z_b, s_a, s_b, zero_s, st_s, t_s, wg_s):
        step = pl.program_id(0)
        nsteps = pl.num_programs(0)

        def ln_rows(top, bot):
            parts = []
            for v in (top, bot):
                w = pltpu.bitcast(v, U32)
                parts.append([_ln(pltpu.bitcast(u, F32)) for u in (w << 16, w & np.uint32(0xFFFF0000))])
            sets = []
            for par in range(2):
                t, b = parts[0][par], parts[1][par]
                x11, x12, x21, x22 = t[:, :D2], t[:, D2:], b[:, :D2], b[:, D2:]
                sets.append(_lhs_combos(x11, x12, x21, x22) + (x12, x21))
            return [pltpu.pack_elementwise([e, o], packed_dtype=BF16) for e, o in zip(*sets)]

        def edges(bb):
            over = x_s[bb, 1, 0:HALO, :]
            for i, c in enumerate(ln_rows(over, jnp.zeros((HALO, D), BF16))):
                xc_s[bb, i, T2 // 2:(T2 + HALO) // 2, :] = c
            xc_s[bb, :, (T2 + HALO) // 2:, :] = jnp.zeros((9, (TP - T2 - HALO) // 2, D2), U32)
            xe = jnp.concatenate([x_s[bb, 0, 0:HALO, :], x_s[bb, 0, T2 - HALO:T2, :], over], axis=0)
            ge = _ln(_gelu(_dot(_ln(xe.astype(F32)).astype(BF16), wup_s[:, D:2 * D])))
            for j in range(NL):
                gi_s[bb, 0, j, 0:HALO, :] = jnp.zeros((HALO, 128), F32)
                gi_s[bb, 0, j, HALO:, :] = ge[0:HALO, j * 128:(j + 1) * 128]
                gi_s[bb, 1, j, :, :] = ge[HALO:, j * 128:(j + 1) * 128]

        def x_copy(bb, r0, r1, n):
            rows = (bb, slice(None), pl.ds(r0, r1 - r0))
            return pltpu.make_async_copy(x_hbm.at[rows], x_s.at[rows], xsem.at[n])

        @pl.when(step == 0)
        def _():
            top, bot = pl.ds(0, D), pl.ds(D, D)
            cp = [pltpu.make_async_copy(s, d, wsem.at[n]) for n, (s, d) in enumerate([
                (wao_hbm, wao_s), (wm_hbm.at[top], wm_s.at[top]), (wv_hbm, wv_s),
                (wq_hbm, wq_s), (wk_hbm, wk_s), (wdn_hbm, wdn_s), (wm_hbm.at[bot], wm_s.at[bot]),
                (dw_hbm, dw_s), (wup_hbm, wup_s)])]
            cuts = [T2 // 16 * n // 4 * 16 for n in range(5)]
            xp = [x_copy(0, cuts[n], cuts[n + 1], n) for n in range(4)]
            stages = [[cp[0], cp[1], xp[0]], [cp[2], xp[1]], [cp[3], cp[4], xp[2]], [cp[5], cp[6], xp[3]],
                      [cp[7], cp[8]]]
            started = [0]

            def arrive(n):
                while started[0] < min(n + 1 + AHEAD, len(stages)):
                    for c in stages[started[0]]:
                        c.start()
                    started[0] += 1
                for c in stages[n]:
                    c.wait()

            def stage(n, dot, lhs_ref, rhs, put):
                nsub = 4
                sub = [cuts[n] + (cuts[n + 1] - cuts[n]) // 16 * k // nsub * 16 for k in range(nsub + 1)]
                wr = D2 // nsub
                for k in range(nsub):
                    lhs = jnp.concatenate([lhs_ref[k * wr:(k + 1) * wr, :],
                                           lhs_ref[D2 + k * wr:D2 + (k + 1) * wr, :]], axis=0)
                    put(k * wr, wr, dot(lhs, rhs()))
                    r0, r1 = sub[k], sub[k + 1]
                    for i, c in enumerate(ln_rows(x_s[0, 0, r0:r1, :], x_s[0, 1, r0:r1, :])):
                        xc_s[0, i, r0 // 2:r1 // 2, :] = c

            def put_plain(r, n, w):
                t_s[r:r + n, :] = w[:n].astype(BF16)
                t_s[D2 + r:D2 + r + n, :] = w[n:].astype(BF16)

            def put_rhs(dst, k0, scale=None):
                def put(r, n, w):
                    if scale is not None:
                        w = w * scale
                    for i, c in enumerate(_rhs_combos(*_quads(w))):
                        dst.bitcast(BF16)[i, k0 + r:k0 + r + n, :] = c.astype(BF16)
                return put

            arrive(0)
            zero_s[...] = jnp.zeros(zero_s.shape, U32)
            gw_b[:, :, h:h + 2 * HALO, :] = jnp.zeros((2, NL, 2 * HALO, 128), F32)
            stage(0, _dot, wao_s, lambda: wm_s[0:D, :], put_plain)
            arrive(1)
            stage(1, _dot, wv_s, lambda: t_s[...], put_rhs(oc_s, 0))
            arrive(2)
            stage(2, _dot_nt, wq_s, lambda: wk_s[...], put_rhs(mc_s, 0, float(D) ** -0.5 * math.log2(math.e)))
            arrive(3)
            stage(3, _dot, wdn_s, lambda: wm_s[D:2 * D, :], put_rhs(oc_s, D2))
            arrive(4)
            x_copy(1, 0, T2, 4).start()
            for r in range(0, D2, 64):
                halves = []
                for r0 in (r, D2 + r):
                    w = pltpu.bitcast(wup_s[r0:r0 + 64, 0:D], U32)
                    halves.append([pltpu.bitcast(u, F32) for u in (w << 16, w & np.uint32(0xFFFF0000))])
                sets = [_rhs_combos(t[:, :D2], t[:, D2:], b[:, :D2], b[:, D2:]) for t, b in zip(*halves)]
                for i, (e, o) in enumerate(zip(*sets)):
                    uc_s[i, r // 2:r // 2 + 32, :] = pltpu.pack_elementwise([e, o], packed_dtype=BF16)
            wg_s[...] = pltpu.bitcast(wup_s[:, D:2 * D], U32)
            dwf = dw_s[...].astype(F32)
            for k in range(K):
                dwb_s[k] = jnp.broadcast_to(dwf[k:k + 1, :], (8, D))
            edges(0)

        first = nt // 2
        nfill = first - 1
        fill_rows = -(-(T2 // 16) // nfill) * 16
        last_rows = T2 - (nfill - 1) * fill_rows

        def fill_store(rows):
            dst = pl.ds(pl.multiple_of((step - 1) * (fill_rows // 2), 8), rows // 2)
            for i in range(9):
                xc_s[1, i, dst, :] = st_s[i, 0:rows // 2, :]

        @pl.when(step == 1)
        def _():
            x_copy(1, 0, T2, 4).wait()

        @pl.when(step == first)
        def _():
            edges(1)

        slot = step % 2
        spare8 = pl.multiple_of(8 * (2 * step // nt), 8)
        clock = [0]
        due = []

        def release(work, todo, val):
            for w in range(todo):
                rr = (h * w // todo) // 8 * 8
                due.append((clock[0] + DLY, work.pop(0)(val[rr:rr + 8, 0:128])))

        def mm(dot, lhs, w):
            bits = None
            due.sort(key=lambda e: e[0])
            while due and due[0][0] <= clock[0]:
                tok = pltpu.bitcast(due.pop(0)[1], U32)
                for a in range(0, tok.shape[0], 8):
                    bits = tok[a:a + 8] if bits is None else bits | tok[a:a + 8]
            if bits is not None:
                head = jnp.concatenate([w[0:8, 0:128] | (bits & zero_s[...]), w[0:8, 128:]], axis=1)
                w = jnp.concatenate([head, w[8:]], axis=0)
            r = dot(lhs, _unpack(w))
            due.append((clock[0] + ORD, r[0:8, 0:128]))
            clock[0] += 1
            return r

        class Tile:
            def __init__(self, t, gw, gw_prev, z, s):
                self.b = t // nt
                self.i = t % nt
                self.r0 = pl.multiple_of(self.i * h, 16)
                self.gw, self.gw_prev, self.z, self.s = gw, gw_prev, z, s
                self.lsum, self.lse, self.pc, self.zc = {}, {}, {}, {}

            def xc(self, i, off):
                rows = pl.ds(pl.multiple_of(self.i * (h // 2) + off // 2, 8), h // 2)
                return xc_s[self.b, i, rows, :]

            def proj(self, w_ref):
                return _seven(lambda i: mm(_dot, _unpack(self.xc(i, 0)), w_ref[i]))

            def proj_g(self):
                xg = jnp.concatenate([
                    jnp.concatenate([self.xc(2, HALO), self.xc(7, HALO)], axis=1),
                    jnp.concatenate([self.xc(8, HALO), self.xc(3, HALO)], axis=1)], axis=0)
                g = _ln(_gelu(_dot(_unpack(xg), _unpack(wg_s[...]))))
                for hf in range(2):
                    for j in range(NL):
                        self.gw[hf, j, 0:2 * HALO, :] = jnp.where(
                            self.i == 0, gi_s[self.b, hf, j], self.gw_prev[hf, j, h:h + 2 * HALO, :])
                        self.gw[hf, j, 2 * HALO:h + 2 * HALO, :] = g[hf * h:(hf + 1) * h, j * 128:(j + 1) * 128]

            def proj_u(self):
                c11, c12, c21, c22 = self.proj(uc_s)
                for hf, (lo, hi) in enumerate(((c11, c12), (c21, c22))):
                    for n in range(2):
                        self.z[hf, n, 0:h, :] = _gelu(lo[:, n * 128:(n + 1) * 128])
                        self.z[hf, 2 + n, 0:h, :] = _gelu(hi[:, n * 128:(n + 1) * 128])

            def proj_q(self):
                q11, q12, q21, q22 = self.proj(mc_s)
                self.qc = [c.astype(BF16) for c in
                           (q11 + q22, q21 + q22, q11, q22, q11 + q12, q21 - q11, q12 - q22)]

            def conv_piece(self, hf, j, a, gate):
                self.gw[hf, j, pl.ds(h + 2 * HALO + spare8, 8), :] = gate
                acc = None
                for k in sorted(range(K), key=lambda k: (k % 8, k)):
                    w = dwb_s[k, :, j * 128:(j + 1) * 128]
                    t = self.gw[hf, j, a + k + 1:a + k + 1 + CR, :].reshape(CR // 8, 8, 128) * w[None]
                    acc = t if acc is None else acc + t
                z = acc.reshape(CR, 128) * self.z[hf, j, a:a + CR, :]
                self.z[hf, j, a:a + CR, :] = z
                return z

            def z_piece(self, a, gate):
                self.z[0, 0, pl.ds(h + spare8, 8), :] = gate
                tiles = [_lhs_combos(*[self.z[hf, 2 * s + n, a:a + 16, :] for hf in range(2) for s in range(2)])
                         for n in range(2)]
                self.zc[a] = [jnp.concatenate([t[i] for t in tiles], axis=1) for i in range(7)]
                return tiles[1][6]

            def conv_pieces(self):
                work = []
                for a in range(0, h, 16):
                    work += [lambda g, hf=hf, j=j, a=r: self.conv_piece(hf, j, a, g)
                             for hf in range(2) for j in range(NL) for r in range(a, a + 16, CR)]
                    work.append(lambda g, a=a: self.z_piece(a, g))
                return work

            def qk(self, work, margin):
                nchunk = TP // QC
                nslots = nchunk * 7 - margin
                total = len(work)
                mx = [None, None]
                cnt = [0]
                src = (0, 2, 1, 4, 3, 5, 6)

                for c in range(nchunk):
                    keys = pl.ds(c * QC // 2, QC // 2)

                    def prod(i):
                        r = mm(_dot_nt, self.qc[i], xc_s[self.b, src[i], keys, :])
                        n = cnt[0]
                        cnt[0] += 1
                        if n < nslots:
                            release(work, (n + 1) * total // nslots - n * total // nslots, r)
                        return r

                    def emit(hf, side, val):
                        for n in range(QC // 128):
                            kt = c * (QC // 128) + n
                            t = val[:, n * 128:(n + 1) * 128]
                            if (kt + 1) * 128 > T2:
                                col = kt * 128 + lax.broadcasted_iota(jnp.int32, (h, 128), 1)
                                t = jnp.where(col < T2, t, -jnp.inf)
                            self.s[hf, side, kt, 0:h, :] = t
                            mx[hf] = t if mx[hf] is None else jnp.maximum(mx[hf], t)

                    if QORD == 0:
                        m2 = prod(1)
                        m4 = prod(3)
                        emit(1, 0, m2 - m4)
                        m1 = prod(0)
                        t11 = m1 - m4
                        t22 = m1 - m2
                        t11 = t11 + prod(6)
                        m5 = prod(4)
                        emit(0, 0, t11 - m5)
                        m3 = prod(2)
                        emit(0, 1, m5 - m3)
                        emit(1, 1, (t22 - m3) + prod(5))
                    elif QORD == 1:
                        t11 = prod(6)
                        m4 = prod(3)
                        t11 = t11 - m4
                        m2 = prod(1)
                        emit(1, 0, m2 - m4)
                        m1 = prod(0)
                        t11 = t11 + m1
                        t22 = m1 - m2
                        m5 = prod(4)
                        emit(0, 0, t11 - m5)
                        m3 = prod(2)
                        emit(0, 1, m5 - m3)
                        emit(1, 1, (t22 - m3) + prod(5))
                self.m = [jnp.max(v, axis=-1, keepdims=True) for v in mx]

            def gate_s(self, gate):
                self.s[0, 0, 0, pl.ds(h + spare8, 8), :] = gate

            def sum_piece(self, hf, a, tiles, last, gate):
                self.gate_s(gate)
                m = self.m[hf][a:a + 16]
                mb = jnp.broadcast_to(m, (16, 128))
                acc = self.lsum.get((hf, a))
                for side, kt in tiles:
                    e = jnp.exp2(self.s[hf, side, kt, a:a + 16, :] - mb)
                    acc = e if acc is None else acc + e
                self.lsum[hf, a] = acc
                if last:
                    l = jnp.sum(acc, axis=-1, keepdims=True)
                    acc = self.lse[hf, a] = jnp.broadcast_to(m + jnp.log2(l), (16, 128))
                return acc

            def sum_pieces(self):
                tiles = [(side, kt) for side in range(2) for kt in range(NKT) if kt * 128 < T2]
                work = []
                for a in range(0, h, 16):
                    work += [lambda g, hf=hf, a=a, n=n: self.sum_piece(hf, a, tiles[n:n + SUMT], n + SUMT >= len(tiles), g)
                             for hf in range(2) for n in range(0, len(tiles), SUMT)]
                    work += [lambda g, kt=kt, a=a: self.exp_piece(kt, a, g) for kt in range(0, PC // 128, EXPT)]
                return work

            def exp_piece(self, kt0, a, gate):
                self.gate_s(gate)
                tok = None
                for kt in range(kt0, kt0 + EXPT):
                    p = [jnp.exp2(self.s[hf, side, kt, a:a + 16, :] - self.lse[hf, a])
                         for hf in range(2) for side in range(2)]
                    cs = self.pc[kt, a] = _lhs_combos(*p)
                    t = cs[5] + cs[6]
                    tok = t if tok is None else tok + t
                return tok

            def exp_pieces(self, c):
                return [lambda g, kt=kt, a=a: self.exp_piece(kt, a, g)
                        for a in range(0, h, 16) for kt in range(c * PC // 128, (c + 1) * PC // 128, EXPT)]

            def pv(self, works):
                src = (0, 2, 6, 5, 3, 4, 1)
                acc = [None] * 7
                for c in range(TP // PC):
                    keys = pl.ds(c * PC // 2, PC // 2)
                    work = works[c]
                    total = len(work)
                    for n, i in enumerate((1, 3, 0, 6, 4, 2, 5)):
                        p = jnp.concatenate([
                            jnp.concatenate([self.pc[kt, a][i] for kt in range(c * PC // 128, (c + 1) * PC // 128)], axis=1)
                            for a in range(0, h, 16)], axis=0).astype(BF16)
                        r = mm(_dot, p, xc_s[self.b, src[i], keys, :])
                        acc[i] = r if acc[i] is None else acc[i] + r
                        if n < 7 - PVM:
                            release(work, (n + 1) * total // (7 - PVM) - n * total // (7 - PVM), acc[i])
                n1, n2, n3, n4, n5, n6, n7 = acc
                self.oc = _lhs_combos(n1 - n4 - n5 - n7, n3 - n5, n4 - n2, n1 - n2 - n3 - n6)

            def out(self, dst):
                zc = [jnp.concatenate([self.zc[a][i] for a in range(0, h, 16)], axis=0) for i in range(7)]
                c11, c12, c21, c22 = _seven(
                    lambda i: mm(_dot, jnp.concatenate([self.oc[i], zc[i]], axis=1).astype(BF16), oc_s[i]))
                for hf, (lo, hi) in enumerate(((c11, c12), (c21, c22))):
                    res = x_s[self.b, hf, pl.ds(self.r0, h), :].astype(F32)
                    o_s[slot, dst, hf] = (jnp.concatenate([lo, hi], axis=1) + res).astype(o_s.dtype)

            def out_copy(self, sl, dst):
                return pltpu.make_async_copy(
                    o_s.at[sl, dst], o_hbm.at[self.b, :, pl.ds(self.r0, h), :], osem.at[sl, dst])

        ta = Tile(2 * step, gw_a, gw_b, z_a, s_a)
        tb = Tile(2 * step + 1, gw_b, gw_a, z_b, s_b)

        @pl.when(step >= 2)
        def _():
            ta.out_copy(slot, 0).wait()
            tb.out_copy(slot, 1).wait()

        npv = TP // PC
        conv = ta.conv_pieces() + tb.conv_pieces()
        cut = [len(conv) * n // sum(SPLIT) for n in np.cumsum((0,) + SPLIT)]
        cw = [conv[cut[n]:cut[n + 1]] for n in range(4)]

        def part(l, c, n):
            return l[c * len(l) // n:(c + 1) * len(l) // n] if c < n else []

        ta.proj_g(); ta.proj_u(); ta.proj_q()
        if not LATE:
            tb.proj_g(); tb.proj_u(); tb.proj_q()
        def fill_piece(n, gate):
            r = jnp.clip((step - 1) * fill_rows + n * 16, 0, T2 - 16)
            rows = pl.ds(pl.multiple_of(r, 16), 16)
            bb = jnp.minimum(step, 1)
            hold = pltpu.bitcast(gate, U32) & zero_s[...]
            top, bot = [_unpack(pltpu.bitcast(x_s[bb, hf, rows, :], U32) | jnp.concatenate([hold] * NL, axis=1))
                        for hf in range(2)]
            cs = ln_rows(top, bot)
            for i, c in enumerate(cs):
                st_s[i, n * 8:n * 8 + 8, :] = c
            return cs[0][:, 0:128]

        fills = [lambda g, n=n: fill_piece(n, g) for n in range(fill_rows // 16)]
        ta.qk(cw[0], 0)
        if LATE:
            tb.proj_g(); tb.proj_u(); tb.proj_q()
        tb.qk(_mix(cw[1], ta.sum_pieces()), QKM)
        sb = tb.sum_pieces()
        cut = [len(sb) * n // sum(SBW) for n in np.cumsum((0,) + SBW)]
        ta.pv([_mix(ta.exp_pieces(c + 1) if c + 1 < npv else [],
                    sb[cut[c]:cut[c + 1]], part(cw[2], c, npv)) for c in range(npv)])
        tb.pv([_mix(tb.exp_pieces(c + 1) if c + 1 < npv else [], part(cw[3], npv - 1 - c, 1),
                    part(fills, c, npv - 1)) for c in range(npv)])
        ta.out(0)
        tb.out(1)
        ta.out_copy(slot, 0).start()
        tb.out_copy(slot, 1).start()

        @pl.when((step >= 1) & (step < nfill))
        def _():
            fill_store(fill_rows)

        @pl.when(step == nfill)
        def _():
            fill_store(last_rows)

        @pl.when(step == nsteps - 1)
        def _():
            ta.out_copy(slot, 0).wait()
            tb.out_copy(slot, 1).wait()
            ta.out_copy(1 - slot, 0).wait()
            tb.out_copy(1 - slot, 1).wait()

    gw_shape = (2, NL, h + 2 * HALO + 16, 128)
    z_shape = (2, NL, h + 16, 128)
    s_shape = (2, 2, NKT, h + 16, 128)
    out = pl.pallas_call(
        kernel,
        grid=(B * nt // 2,),
        in_specs=[pl.BlockSpec(memory_space=pl.ANY)] * 9,
        out_specs=pl.BlockSpec(memory_space=pl.ANY),
        out_shape=jax.ShapeDtypeStruct((B, 2, T2, D), x.dtype),
        scratch_shapes=[
            pltpu.VMEM((B, 2, T2, D), BF16),
            pltpu.VMEM((D, D), BF16), pltpu.VMEM((D, D), BF16), pltpu.VMEM((D, D), BF16), pltpu.VMEM((D, D), BF16),
            pltpu.VMEM((D, 2 * D), BF16), pltpu.VMEM((K, D), BF16), pltpu.VMEM((D, D), BF16), pltpu.VMEM((2 * D, D), BF16),
            pltpu.SemaphoreType.DMA((9,)), pltpu.SemaphoreType.DMA((5,)), pltpu.SemaphoreType.DMA((2, 2)),
            pltpu.VMEM((7, D2 // 2, D2), U32), pltpu.VMEM((7, D2 // 2, D2), U32), pltpu.VMEM((7, D2, D2), U32),
            pltpu.VMEM((K, 8, D), F32),
            pltpu.VMEM((B, 9, TP // 2, D2), U32),
            pltpu.VMEM((B, 2, NL, 2 * HALO, 128), F32),
            pltpu.VMEM((2, 2, 2, h, D), x.dtype),
            pltpu.VMEM(gw_shape, F32), pltpu.VMEM(gw_shape, F32),
            pltpu.VMEM(z_shape, F32), pltpu.VMEM(z_shape, F32),
            pltpu.VMEM(s_shape, F32), pltpu.VMEM(s_shape, F32),
            pltpu.VMEM((8, 128), U32),
            pltpu.VMEM((9, -(-(T2 // 16) // (nt // 2 - 1)) * 8, D2), U32),
            pltpu.VMEM((D, D), BF16), pltpu.VMEM((D2, D), U32),
        ],
        compiler_params=pltpu.CompilerParams(
            dimension_semantics=("arbitrary",),
            vmem_limit_bytes=100 * 1024 * 1024, flags=FLAGS, disable_bounds_checks=NOBC,
        ),
    )(x.reshape(B, 2, T2, D), w_q, w_k, w_v, w_ao, w_up, dw, w_dn, w_merge)
    return out.reshape(B, T, D)
```

```python
import math
import numpy as np
import jax
import jax.numpy as jnp
from jax import lax
import jax.experimental.pallas as pl
import jax.experimental.pallas.tpu as pltpu

H = 80
QC = 256
PC = 512
LB = 80
AHEAD = 2
CR = 16
DLY = 6
ORD = 3
SUMT = 8
EXPT = 2
SPLIT = (55, 15, 5, 15)
QKM = 4
PVM = 1
SBW = (1, 1, 1, 2)
NOBC = True
LATE = False
QORD = 1
NSUB = 2
LSUB = 6
FLAGS = None
F32 = jnp.float32
BF16 = jnp.bfloat16
U32 = jnp.uint32


def _dot(a, b):
    return jnp.dot(a, b, preferred_element_type=F32)


def _dot_nt(a, b):
    return lax.dot_general(a, b, (((1,), (1,)), ((), ())), preferred_element_type=F32)


def _pack(v):
    return pltpu.bitcast(v.astype(BF16), U32)


def _unpack(w):
    return pltpu.bitcast(w, BF16)


def _ln(x):
    m = jnp.mean(x, axis=-1, keepdims=True)
    xc = x - m
    v = jnp.mean(xc * xc, axis=-1, keepdims=True)
    return xc * lax.rsqrt(v + 1e-5)


def _gelu(x):
    c = math.sqrt(2.0 / math.pi)
    hx = 0.5 * x
    return hx + hx * jnp.tanh(x * (c + (c * 0.044715) * (x * x)))


def _lhs_combos(a11, a12, a21, a22):
    return (a11 + a22, a22 - a21, a11, a22, a11 - a12, a21 + a11, a12 + a22)


def _rhs_combos(b11, b12, b21, b22):
    return (b11 + b22, b11, b12 + b22, b21 + b11, b22, b12 - b11, b21 - b22)


def _quads(w):
    r, c = w.shape[0] // 2, w.shape[1] // 2
    return w[:r, :c], w[:r, c:], w[r:, :c], w[r:, c:]


def _seven(prod):
    n2 = prod(1)
    n4 = prod(3)
    c21 = n4 - n2
    n1 = prod(0)
    t11 = n1 - n4
    t22 = n1 - n2
    t11 = t11 + prod(6)
    n5 = prod(4)
    c11 = t11 - n5
    n3 = prod(2)
    c12 = n3 - n5
    c22 = (t22 - n3) + prod(5)
    return c11, c12, c21, c22


def _mix(*lists):
    keyed = [((n + 0.5) / len(l), k, n, w) for k, l in enumerate(lists) for n, w in enumerate(l)]
    return [e[3] for e in sorted(keyed, key=lambda e: e[:3])]


@jax.jit
def pallas_standalone__conformer_family_branchformer__speech_kernel(
    x, w_q, w_k, w_v, w_ao, w_up, dw, w_dn, w_merge,
):
    B, T, D = x.shape
    K = dw.shape[0]
    T2 = T // 2
    D2 = D // 2
    h = H
    nt = T2 // h
    TP = -(-T2 // PC) * PC
    NKT = TP // 128
    HALO = 16
    NL = D // 128
    assert B == 2 and (B * nt) % 2 == 0 and T2 % h == 0 and T2 % LB == 0 and TP >= T2 + HALO

    def kernel(x_hbm, wq_hbm, wk_hbm, wv_hbm, wao_hbm, wup_hbm, dw_hbm, wdn_hbm, wm_hbm, o_hbm,
               x_s, wq_s, wk_s, wv_s, wao_s, wup_s, dw_s, wdn_s, wm_s, wsem, xsem, osem,
               mc_s, uc_s, oc_s, dwb_s, xc_s, gi_s, o_s,
               gw_a, gw_b, z_a, z_b, s_a, s_b, zero_s, st_s, t_s, wg_s):
        step = pl.program_id(0)
        nsteps = pl.num_programs(0)

        def ln_rows(top, bot):
            t, b = _ln(top.astype(F32)), _ln(bot.astype(F32))
            x11, x12, x21, x22 = t[:, :D2], t[:, D2:], b[:, :D2], b[:, D2:]
            return [_pack(c) for c in _lhs_combos(x11, x12, x21, x22) + (x12, x21)]

        def edges(bb):
            over = x_s[bb, 1, 0:HALO, :]
            for i, c in enumerate(ln_rows(over, jnp.zeros((HALO, D), BF16))):
                xc_s[bb, i, T2 // 2:(T2 + HALO) // 2, :] = c
            xc_s[bb, :, (T2 + HALO) // 2:, :] = jnp.zeros((9, (TP - T2 - HALO) // 2, D2), U32)
            xe = jnp.concatenate([x_s[bb, 0, 0:HALO, :], x_s[bb, 0, T2 - HALO:T2, :], over], axis=0)
            ge = _ln(_gelu(_dot(_ln(xe.astype(F32)).astype(BF16), wup_s[:, D:2 * D])))
            for j in range(NL):
                gi_s[bb, 0, j, 0:HALO, :] = jnp.zeros((HALO, 128), F32)
                gi_s[bb, 0, j, HALO:, :] = ge[0:HALO, j * 128:(j + 1) * 128]
                gi_s[bb, 1, j, :, :] = ge[HALO:, j * 128:(j + 1) * 128]

        def x_copy(bb, r0, r1, n):
            rows = (bb, slice(None), pl.ds(r0, r1 - r0))
            return pltpu.make_async_copy(x_hbm.at[rows], x_s.at[rows], xsem.at[n])

        @pl.when(step == 0)
        def _():
            top, bot = pl.ds(0, D), pl.ds(D, D)
            cp = [pltpu.make_async_copy(s, d, wsem.at[n]) for n, (s, d) in enumerate([
                (wao_hbm, wao_s), (wm_hbm.at[top], wm_s.at[top]), (wv_hbm, wv_s),
                (wq_hbm, wq_s), (wk_hbm, wk_s), (wdn_hbm, wdn_s), (wm_hbm.at[bot], wm_s.at[bot]),
                (dw_hbm, dw_s), (wup_hbm, wup_s)])]
            cuts = [T2 // 16 * n // 4 * 16 for n in range(5)]
            xp = [x_copy(0, cuts[n], cuts[n + 1], n) for n in range(4)]
            stages = [[cp[0], cp[1], xp[0]], [cp[2], xp[1]], [cp[3], cp[4], xp[2]], [cp[5], cp[6], xp[3]],
                      [cp[7], cp[8]]]
            started = [0]

            def arrive(n):
                while started[0] < min(n + 1 + AHEAD, len(stages)):
                    for c in stages[started[0]]:
                        c.start()
                    started[0] += 1
                for c in stages[n]:
                    c.wait()

            def stage(n, dot, lhs_ref, rhs, put):
                sub = [cuts[n] + (cuts[n + 1] - cuts[n]) // 16 * k // (NSUB * LSUB) * 16 for k in range(NSUB * LSUB + 1)]
                wr = D2 // NSUB
                for k in range(NSUB):
                    lhs = jnp.concatenate([lhs_ref[k * wr:(k + 1) * wr, :],
                                           lhs_ref[D2 + k * wr:D2 + (k + 1) * wr, :]], axis=0)
                    put(k * wr, wr, dot(lhs, rhs()))
                    for r0, r1 in zip(sub[k * LSUB:(k + 1) * LSUB], sub[k * LSUB + 1:]):
                        for i, c in enumerate(ln_rows(x_s[0, 0, r0:r1, :], x_s[0, 1, r0:r1, :])):
                            xc_s[0, i, r0 // 2:r1 // 2, :] = c

            def put_plain(r, n, w):
                t_s[r:r + n, :] = w[:n].astype(BF16)
                t_s[D2 + r:D2 + r + n, :] = w[n:].astype(BF16)

            def put_rhs(dst, k0, scale=None):
                def put(r, n, w):
                    if scale is not None:
                        w = w * scale
                    for i, c in enumerate(_rhs_combos(*_quads(w))):
                        dst[i, (k0 + r) // 2:(k0 + r + n) // 2, :] = _pack(c)
                return put

            arrive(0)
            zero_s[...] = jnp.zeros(zero_s.shape, U32)
            gw_b[:, :, h:h + 2 * HALO, :] = jnp.zeros((2, NL, 2 * HALO, 128), F32)
            stage(0, _dot, wao_s, lambda: wm_s[0:D, :], put_plain)
            arrive(1)
            stage(1, _dot, wv_s, lambda: t_s[...], put_rhs(oc_s, 0))
            arrive(2)
            stage(2, _dot_nt, wq_s, lambda: wk_s[...], put_rhs(mc_s, 0, float(D) ** -0.5 * math.log2(math.e)))
            arrive(3)
            stage(3, _dot, wdn_s, lambda: wm_s[D:2 * D, :], put_rhs(oc_s, D2))
            arrive(4)
            x_copy(1, 0, T2, 4).start()
            for r in range(0, D2, 64):
                w = jnp.concatenate([wup_s[r:r + 64, 0:D], wup_s[D2 + r:D2 + r + 64, 0:D]], axis=0)
                put_rhs(uc_s, 0)(r, 64, w.astype(F32))
            wg_s[...] = pltpu.bitcast(wup_s[:, D:2 * D], U32)
            dwf = dw_s[...].astype(F32)
            for k in range(K):
                dwb_s[k] = jnp.broadcast_to(dwf[k:k + 1, :], (8, D))
            edges(0)

        first = nt // 2
        nfill = first - 1
        fill_rows = -(-(T2 // 16) // nfill) * 16
        last_rows = T2 - (nfill - 1) * fill_rows

        def fill_store(rows):
            dst = pl.ds(pl.multiple_of((step - 1) * (fill_rows // 2), 8), rows // 2)
            for i in range(9):
                xc_s[1, i, dst, :] = st_s[i, 0:rows // 2, :]

        @pl.when(step == 1)
        def _():
            x_copy(1, 0, T2, 4).wait()

        @pl.when(step == first)
        def _():
            edges(1)

        slot = step % 2
        spare8 = pl.multiple_of(8 * (2 * step // nt), 8)
        clock = [0]
        due = []

        def release(work, todo, val):
            for w in range(todo):
                rr = (h * w // todo) // 8 * 8
                due.append((clock[0] + DLY, work.pop(0)(val[rr:rr + 8, 0:128])))

        def mm(dot, lhs, w):
            bits = None
            due.sort(key=lambda e: e[0])
            while due and due[0][0] <= clock[0]:
                tok = pltpu.bitcast(due.pop(0)[1], U32)
                for a in range(0, tok.shape[0], 8):
                    bits = tok[a:a + 8] if bits is None else bits | tok[a:a + 8]
            if bits is not None:
                head = jnp.concatenate([w[0:8, 0:128] | (bits & zero_s[...]), w[0:8, 128:]], axis=1)
                w = jnp.concatenate([head, w[8:]], axis=0)
            r = dot(lhs, _unpack(w))
            due.append((clock[0] + ORD, r[0:8, 0:128]))
            clock[0] += 1
            return r

        class Tile:
            def __init__(self, t, gw, gw_prev, z, s):
                self.b = t // nt
                self.i = t % nt
                self.r0 = pl.multiple_of(self.i * h, 16)
                self.gw, self.gw_prev, self.z, self.s = gw, gw_prev, z, s
                self.lsum, self.lse, self.pc, self.zc = {}, {}, {}, {}

            def xc(self, i, off):
                rows = pl.ds(pl.multiple_of(self.i * (h // 2) + off // 2, 8), h // 2)
                return xc_s[self.b, i, rows, :]

            def proj(self, w_ref):
                return _seven(lambda i: mm(_dot, _unpack(self.xc(i, 0)), w_ref[i]))

            def proj_g(self):
                xg = jnp.concatenate([
                    jnp.concatenate([self.xc(2, HALO), self.xc(7, HALO)], axis=1),
                    jnp.concatenate([self.xc(8, HALO), self.xc(3, HALO)], axis=1)], axis=0)
                g = _ln(_gelu(_dot(_unpack(xg), _unpack(wg_s[...]))))
                for hf in range(2):
                    for j in range(NL):
                        self.gw[hf, j, 0:2 * HALO, :] = jnp.where(
                            self.i == 0, gi_s[self.b, hf, j], self.gw_prev[hf, j, h:h + 2 * HALO, :])
                        self.gw[hf, j, 2 * HALO:h + 2 * HALO, :] = g[hf * h:(hf + 1) * h, j * 128:(j + 1) * 128]

            def proj_u(self):
                c11, c12, c21, c22 = self.proj(uc_s)
                for hf, (lo, hi) in enumerate(((c11, c12), (c21, c22))):
                    for n in range(2):
                        self.z[hf, n, 0:h, :] = _gelu(lo[:, n * 128:(n + 1) * 128])
                        self.z[hf, 2 + n, 0:h, :] = _gelu(hi[:, n * 128:(n + 1) * 128])

            def proj_q(self):
                q11, q12, q21, q22 = self.proj(mc_s)
                self.qc = [c.astype(BF16) for c in
                           (q11 + q22, q21 + q22, q11, q22, q11 + q12, q21 - q11, q12 - q22)]

            def conv_piece(self, hf, j, a, gate):
                self.gw[hf, j, pl.ds(h + 2 * HALO + spare8, 8), :] = gate
                acc = None
                for k in sorted(range(K), key=lambda k: (k % 8, k)):
                    w = dwb_s[k, :, j * 128:(j + 1) * 128]
                    t = self.gw[hf, j, a + k + 1:a + k + 1 + CR, :].reshape(CR // 8, 8, 128) * w[None]
                    acc = t if acc is None else acc + t
                z = acc.reshape(CR, 128) * self.z[hf, j, a:a + CR, :]
                self.z[hf, j, a:a + CR, :] = z
                return z

            def z_piece(self, a, gate):
                self.z[0, 0, pl.ds(h + spare8, 8), :] = gate
                tiles = [_lhs_combos(*[self.z[hf, 2 * s + n, a:a + 16, :] for hf in range(2) for s in range(2)])
                         for n in range(2)]
                self.zc[a] = [jnp.concatenate([t[i] for t in tiles], axis=1) for i in range(7)]
                return tiles[1][6]

            def conv_pieces(self):
                work = []
                for a in range(0, h, 16):
                    work += [lambda g, hf=hf, j=j, a=r: self.conv_piece(hf, j, a, g)
                             for hf in range(2) for j in range(NL) for r in range(a, a + 16, CR)]
                    work.append(lambda g, a=a: self.z_piece(a, g))
                return work

            def qk(self, work, margin):
                nchunk = TP // QC
                nslots = nchunk * 7 - margin
                total = len(work)
                mx = [None, None]
                cnt = [0]
                src = (0, 2, 1, 4, 3, 5, 6)

                for c in range(nchunk):
                    keys = pl.ds(c * QC // 2, QC // 2)

                    def prod(i):
                        r = mm(_dot_nt, self.qc[i], xc_s[self.b, src[i], keys, :])
                        n = cnt[0]
                        cnt[0] += 1
                        if n < nslots:
                            release(work, (n + 1) * total // nslots - n * total // nslots, r)
                        return r

                    def emit(hf, side, val):
                        for n in range(QC // 128):
                            kt = c * (QC // 128) + n
                            t = val[:, n * 128:(n + 1) * 128]
                            if (kt + 1) * 128 > T2:
                                col = kt * 128 + lax.broadcasted_iota(jnp.int32, (h, 128), 1)
                                t = jnp.where(col < T2, t, -jnp.inf)
                            self.s[hf, side, kt, 0:h, :] = t
                            mx[hf] = t if mx[hf] is None else jnp.maximum(mx[hf], t)

                    if QORD == 0:
                        m2 = prod(1)
                        m4 = prod(3)
                        emit(1, 0, m2 - m4)
                        m1 = prod(0)
                        t11 = m1 - m4
                        t22 = m1 - m2
                        t11 = t11 + prod(6)
                        m5 = prod(4)
                        emit(0, 0, t11 - m5)
                        m3 = prod(2)
                        emit(0, 1, m5 - m3)
                        emit(1, 1, (t22 - m3) + prod(5))
                    elif QORD == 1:
                        t11 = prod(6)
                        m4 = prod(3)
                        t11 = t11 - m4
                        m2 = prod(1)
                        emit(1, 0, m2 - m4)
                        m1 = prod(0)
                        t11 = t11 + m1
                        t22 = m1 - m2
                        m5 = prod(4)
                        emit(0, 0, t11 - m5)
                        m3 = prod(2)
                        emit(0, 1, m5 - m3)
                        emit(1, 1, (t22 - m3) + prod(5))
                self.m = [jnp.max(v, axis=-1, keepdims=True) for v in mx]

            def gate_s(self, gate):
                self.s[0, 0, 0, pl.ds(h + spare8, 8), :] = gate

            def sum_piece(self, hf, a, tiles, last, gate):
                self.gate_s(gate)
                m = self.m[hf][a:a + 16]
                mb = jnp.broadcast_to(m, (16, 128))
                acc = self.lsum.get((hf, a))
                for side, kt in tiles:
                    e = jnp.exp2(self.s[hf, side, kt, a:a + 16, :] - mb)
                    acc = e if acc is None else acc + e
                self.lsum[hf, a] = acc
                if last:
                    l = jnp.sum(acc, axis=-1, keepdims=True)
                    acc = self.lse[hf, a] = jnp.broadcast_to(m + jnp.log2(l), (16, 128))
                return acc

            def sum_pieces(self):
                tiles = [(side, kt) for side in range(2) for kt in range(NKT) if kt * 128 < T2]
                work = []
                for a in range(0, h, 16):
                    work += [lambda g, hf=hf, a=a, n=n: self.sum_piece(hf, a, tiles[n:n + SUMT], n + SUMT >= len(tiles), g)
                             for hf in range(2) for n in range(0, len(tiles), SUMT)]
                    work += [lambda g, kt=kt, a=a: self.exp_piece(kt, a, g) for kt in range(0, PC // 128, EXPT)]
                return work

            def exp_piece(self, kt0, a, gate):
                self.gate_s(gate)
                tok = None
                for kt in range(kt0, kt0 + EXPT):
                    p = [jnp.exp2(self.s[hf, side, kt, a:a + 16, :] - self.lse[hf, a])
                         for hf in range(2) for side in range(2)]
                    cs = self.pc[kt, a] = _lhs_combos(*p)
                    t = cs[5] + cs[6]
                    tok = t if tok is None else tok + t
                return tok

            def exp_pieces(self, c):
                return [lambda g, kt=kt, a=a: self.exp_piece(kt, a, g)
                        for a in range(0, h, 16) for kt in range(c * PC // 128, (c + 1) * PC // 128, EXPT)]

            def pv(self, works):
                src = (0, 2, 6, 5, 3, 4, 1)
                acc = [None] * 7
                for c in range(TP // PC):
                    keys = pl.ds(c * PC // 2, PC // 2)
                    work = works[c]
                    total = len(work)
                    for n, i in enumerate((1, 3, 0, 6, 4, 2, 5)):
                        p = jnp.concatenate([
                            jnp.concatenate([self.pc[kt, a][i] for kt in range(c * PC // 128, (c + 1) * PC // 128)], axis=1)
                            for a in range(0, h, 16)], axis=0).astype(BF16)
                        r = mm(_dot, p, xc_s[self.b, src[i], keys, :])
                        acc[i] = r if acc[i] is None else acc[i] + r
                        if n < 7 - PVM:
                            release(work, (n + 1) * total // (7 - PVM) - n * total // (7 - PVM), acc[i])
                n1, n2, n3, n4, n5, n6, n7 = acc
                self.oc = _lhs_combos(n1 - n4 - n5 - n7, n3 - n5, n4 - n2, n1 - n2 - n3 - n6)

            def out(self, dst):
                zc = [jnp.concatenate([self.zc[a][i] for a in range(0, h, 16)], axis=0) for i in range(7)]
                c11, c12, c21, c22 = _seven(
                    lambda i: mm(_dot, jnp.concatenate([self.oc[i], zc[i]], axis=1).astype(BF16), oc_s[i]))
                for hf, (lo, hi) in enumerate(((c11, c12), (c21, c22))):
                    res = x_s[self.b, hf, pl.ds(self.r0, h), :].astype(F32)
                    o_s[slot, dst, hf] = (jnp.concatenate([lo, hi], axis=1) + res).astype(o_s.dtype)

            def out_copy(self, sl, dst):
                return pltpu.make_async_copy(
                    o_s.at[sl, dst], o_hbm.at[self.b, :, pl.ds(self.r0, h), :], osem.at[sl, dst])

        ta = Tile(2 * step, gw_a, gw_b, z_a, s_a)
        tb = Tile(2 * step + 1, gw_b, gw_a, z_b, s_b)

        @pl.when(step >= 2)
        def _():
            ta.out_copy(slot, 0).wait()
            tb.out_copy(slot, 1).wait()

        npv = TP // PC
        conv = ta.conv_pieces() + tb.conv_pieces()
        cut = [len(conv) * n // sum(SPLIT) for n in np.cumsum((0,) + SPLIT)]
        cw = [conv[cut[n]:cut[n + 1]] for n in range(4)]

        def part(l, c, n):
            return l[c * len(l) // n:(c + 1) * len(l) // n] if c < n else []

        ta.proj_g(); ta.proj_u(); ta.proj_q()
        if not LATE:
            tb.proj_g(); tb.proj_u(); tb.proj_q()
        def fill_piece(n, gate):
            r = jnp.clip((step - 1) * fill_rows + n * 16, 0, T2 - 16)
            rows = pl.ds(pl.multiple_of(r, 16), 16)
            bb = jnp.minimum(step, 1)
            hold = pltpu.bitcast(gate, U32) & zero_s[...]
            top, bot = [_unpack(pltpu.bitcast(x_s[bb, hf, rows, :], U32) | jnp.concatenate([hold] * NL, axis=1))
                        for hf in range(2)]
            cs = ln_rows(top, bot)
            for i, c in enumerate(cs):
                st_s[i, n * 8:n * 8 + 8, :] = c
            return cs[0][:, 0:128]

        fills = [lambda g, n=n: fill_piece(n, g) for n in range(fill_rows // 16)]
        ta.qk(cw[0], 0)
        if LATE:
            tb.proj_g(); tb.proj_u(); tb.proj_q()
        tb.qk(_mix(cw[1], ta.sum_pieces()), QKM)
        sb = tb.sum_pieces()
        cut = [len(sb) * n // sum(SBW) for n in np.cumsum((0,) + SBW)]
        ta.pv([_mix(ta.exp_pieces(c + 1) if c + 1 < npv else [],
                    sb[cut[c]:cut[c + 1]], part(cw[2], c, npv)) for c in range(npv)])
        tb.pv([_mix(tb.exp_pieces(c + 1) if c + 1 < npv else [], part(cw[3], npv - 1 - c, 1),
                    part(fills, c, npv - 1)) for c in range(npv)])
        ta.out(0)
        tb.out(1)
        ta.out_copy(slot, 0).start()
        tb.out_copy(slot, 1).start()

        @pl.when((step >= 1) & (step < nfill))
        def _():
            fill_store(fill_rows)

        @pl.when(step == nfill)
        def _():
            fill_store(last_rows)

        @pl.when(step == nsteps - 1)
        def _():
            ta.out_copy(slot, 0).wait()
            tb.out_copy(slot, 1).wait()
            ta.out_copy(1 - slot, 0).wait()
            tb.out_copy(1 - slot, 1).wait()

    gw_shape = (2, NL, h + 2 * HALO + 16, 128)
    z_shape = (2, NL, h + 16, 128)
    s_shape = (2, 2, NKT, h + 16, 128)
    out = pl.pallas_call(
        kernel,
        grid=(B * nt // 2,),
        in_specs=[pl.BlockSpec(memory_space=pl.ANY)] * 9,
        out_specs=pl.BlockSpec(memory_space=pl.ANY),
        out_shape=jax.ShapeDtypeStruct((B, 2, T2, D), x.dtype),
        scratch_shapes=[
            pltpu.VMEM((B, 2, T2, D), BF16),
            pltpu.VMEM((D, D), BF16), pltpu.VMEM((D, D), BF16), pltpu.VMEM((D, D), BF16), pltpu.VMEM((D, D), BF16),
            pltpu.VMEM((D, 2 * D), BF16), pltpu.VMEM((K, D), BF16), pltpu.VMEM((D, D), BF16), pltpu.VMEM((2 * D, D), BF16),
            pltpu.SemaphoreType.DMA((9,)), pltpu.SemaphoreType.DMA((5,)), pltpu.SemaphoreType.DMA((2, 2)),
            pltpu.VMEM((7, D2 // 2, D2), U32), pltpu.VMEM((7, D2 // 2, D2), U32), pltpu.VMEM((7, D2, D2), U32),
            pltpu.VMEM((K, 8, D), F32),
            pltpu.VMEM((B, 9, TP // 2, D2), U32),
            pltpu.VMEM((B, 2, NL, 2 * HALO, 128), F32),
            pltpu.VMEM((2, 2, 2, h, D), x.dtype),
            pltpu.VMEM(gw_shape, F32), pltpu.VMEM(gw_shape, F32),
            pltpu.VMEM(z_shape, F32), pltpu.VMEM(z_shape, F32),
            pltpu.VMEM(s_shape, F32), pltpu.VMEM(s_shape, F32),
            pltpu.VMEM((8, 128), U32),
            pltpu.VMEM((9, -(-(T2 // 16) // (nt // 2 - 1)) * 8, D2), U32),
            pltpu.VMEM((D, D), BF16), pltpu.VMEM((D2, D), U32),
        ],
        compiler_params=pltpu.CompilerParams(
            dimension_semantics=("arbitrary",),
            vmem_limit_bytes=100 * 1024 * 1024, flags=FLAGS, disable_bounds_checks=NOBC,
        ),
    )(x.reshape(B, 2, T2, D), w_q, w_k, w_v, w_ao, w_up, dw, w_dn, w_merge)
    return out.reshape(B, T, D)
```

```python
import math

import jax
import jax.experimental.pallas as pl
import jax.experimental.pallas.tpu as pltpu
import jax.numpy as jnp
import numpy as np
from jax import lax

F32 = jnp.float32
BF16 = jnp.bfloat16
U32 = jnp.uint32

H = 80
QC = 256
PC = 512
HALO = 16
EPS = 1e-5

DLY = 6
ORD = 3
SUMT = 8
EXPT = 2
SPLIT = (55, 15, 5, 15)
SUM_B = (1, 1, 1, 2)
QK_MARGIN = 6
PV_MARGIN = 1


def _dot(a, b):
    return jnp.dot(a, b, preferred_element_type=F32)


def _dot_nt(a, b):
    return lax.dot_general(a, b, (((1,), (1,)), ((), ())), preferred_element_type=F32)


def _pack(v):
    return pltpu.bitcast(v.astype(BF16), U32)


def _unpack(w):
    return pltpu.bitcast(w, BF16)


def _ln(x):
    m = jnp.mean(x, axis=-1, keepdims=True)
    xc = x - m
    v = jnp.mean(xc * xc, axis=-1, keepdims=True)
    return xc * lax.rsqrt(v + EPS)


def _gelu(x):
    c = math.sqrt(2.0 / math.pi)
    hx = 0.5 * x
    return hx + hx * jnp.tanh(x * (c + (c * 0.044715) * (x * x)))


def _lhs_combos(a11, a12, a21, a22):
    return (a11 + a22, a22 - a21, a11, a22, a11 - a12, a21 + a11, a12 + a22)


def _rhs_combos(b11, b12, b21, b22):
    return (b11 + b22, b11, b12 + b22, b21 + b11, b22, b12 - b11, b21 - b22)


def _quads(w):
    r, c = w.shape[0] // 2, w.shape[1] // 2
    return w[:r, :c], w[:r, c:], w[r:, :c], w[r:, c:]


def _seven(prod):
    n2 = prod(1)
    n4 = prod(3)
    c21 = n4 - n2
    n1 = prod(0)
    t11 = n1 - n4
    t22 = n1 - n2
    t11 = t11 + prod(6)
    n5 = prod(4)
    c11 = t11 - n5
    n3 = prod(2)
    c12 = n3 - n5
    c22 = (t22 - n3) + prod(5)
    return c11, c12, c21, c22


def _mix(*lists):
    keyed = [((n + 0.5) / len(l), k, n, w) for k, l in enumerate(lists) for n, w in enumerate(l)]
    return [e[3] for e in sorted(keyed, key=lambda e: e[:3])]


def _share(items, weights):
    cut = [len(items) * int(n) // sum(weights) for n in np.cumsum((0,) + tuple(weights))]
    return [items[a:b] for a, b in zip(cut, cut[1:])]


@jax.jit
def pallas_standalone__conformer_family_branchformer__speech_kernel(
    x: jax.Array,
    w_q: jax.Array,
    w_k: jax.Array,
    w_v: jax.Array,
    w_ao: jax.Array,
    w_up: jax.Array,
    dw: jax.Array,
    w_dn: jax.Array,
    w_merge: jax.Array,
):
    B, T, D = x.shape
    K = dw.shape[0]
    T2 = T // 2
    D2 = D // 2
    NL = D // 128
    h = H
    nt = T2 // h
    TP = -(-T2 // PC) * PC
    NKT = TP // 128
    npv = TP // PC
    first = nt // 2
    nfill = first - 1
    fill_rows = -(-(T2 // 16) // nfill) * 16
    last_rows = T2 - (nfill - 1) * fill_rows
    assert B == 2 and T2 % h == 0 and TP >= T2 + HALO and K == 2 * HALO - 1 and last_rows > 0

    def kernel(x_hbm, wq_hbm, wk_hbm, wv_hbm, wao_hbm, wup_hbm, dw_hbm, wdn_hbm, wm_hbm, o_hbm,
               x_s, wq_s, wk_s, wv_s, wao_s, wup_s, dw_s, wdn_s, wm_s, wsem, xsem, osem,
               mc_s, uc_s, oc_s, dwb_s, xc_s, gi_s, o_s,
               gw_a, gw_b, z_a, z_b, s_a, s_b, zero_s, st_s, t_s, wg_s):
        step = pl.program_id(0)
        nsteps = pl.num_programs(0)

        def ln_rows(top, bot):
            t, b = _ln(top.astype(F32)), _ln(bot.astype(F32))
            x11, x12, x21, x22 = t[:, :D2], t[:, D2:], b[:, :D2], b[:, D2:]
            return [_pack(c) for c in _lhs_combos(x11, x12, x21, x22) + (x12, x21)]

        def edges(bb):
            over = x_s[bb, 1, 0:HALO, :]
            for i, c in enumerate(ln_rows(over, jnp.zeros((HALO, D), BF16))):
                xc_s[bb, i, T2 // 2:(T2 + HALO) // 2, :] = c
            xc_s[bb, :, (T2 + HALO) // 2:, :] = jnp.zeros((9, (TP - T2 - HALO) // 2, D2), U32)
            xe = jnp.concatenate([x_s[bb, 0, 0:HALO, :], x_s[bb, 0, T2 - HALO:T2, :], over], axis=0)
            ge = _ln(_gelu(_dot(_ln(xe.astype(F32)).astype(BF16), wup_s[:, D:2 * D])))
            for j in range(NL):
                gi_s[bb, 0, j, 0:HALO, :] = jnp.zeros((HALO, 128), F32)
                gi_s[bb, 0, j, HALO:, :] = ge[0:HALO, j * 128:(j + 1) * 128]
                gi_s[bb, 1, j, :, :] = ge[HALO:, j * 128:(j + 1) * 128]

        def x_copy(bb, r0, r1, n):
            rows = (bb, slice(None), pl.ds(r0, r1 - r0))
            return pltpu.make_async_copy(x_hbm.at[rows], x_s.at[rows], xsem.at[n])

        @pl.when(step == 0)
        def _():
            top, bot = pl.ds(0, D), pl.ds(D, D)
            cp = [pltpu.make_async_copy(s, d, wsem.at[n]) for n, (s, d) in enumerate([
                (wao_hbm, wao_s), (wm_hbm.at[top], wm_s.at[top]), (wv_hbm, wv_s),
                (wq_hbm, wq_s), (wk_hbm, wk_s), (wdn_hbm, wdn_s), (wm_hbm.at[bot], wm_s.at[bot]),
                (dw_hbm, dw_s), (wup_hbm, wup_s)])]
            cuts = [T2 // 16 * n // 4 * 16 for n in range(5)]
            xp = [x_copy(0, cuts[n], cuts[n + 1], n) for n in range(4)]
            stages = [[cp[0], cp[1], xp[0]], [cp[2], xp[1]], [cp[3], cp[4], xp[2]], [cp[5], cp[6], xp[3]],
                      [cp[7], cp[8]]]
            started = []

            def arrive(n):
                while len(started) < min(n + 3, len(stages)):
                    for c in stages[len(started)]:
                        c.start()
                    started.append(True)
                for c in stages[n]:
                    c.wait()

            def stage(n, dot, lhs_ref, rhs, put):
                sub = [cuts[n] + (cuts[n + 1] - cuts[n]) // 16 * k // 12 * 16 for k in range(13)]
                wr = D2 // 2
                for k in range(2):
                    lhs = jnp.concatenate([lhs_ref[k * wr:(k + 1) * wr, :],
                                           lhs_ref[D2 + k * wr:D2 + (k + 1) * wr, :]], axis=0)
                    put(k * wr, wr, dot(lhs, rhs()))
                    for r0, r1 in zip(sub[k * 6:(k + 1) * 6], sub[k * 6 + 1:]):
                        for i, c in enumerate(ln_rows(x_s[0, 0, r0:r1, :], x_s[0, 1, r0:r1, :])):
                            xc_s[0, i, r0 // 2:r1 // 2, :] = c

            def put_plain(r, n, w):
                t_s[r:r + n, :] = w[:n].astype(BF16)
                t_s[D2 + r:D2 + r + n, :] = w[n:].astype(BF16)

            def put_rhs(dst, k0, scale=None):
                def put(r, n, w):
                    if scale is not None:
                        w = w * scale
                    for i, c in enumerate(_rhs_combos(*_quads(w))):
                        dst[i, (k0 + r) // 2:(k0 + r + n) // 2, :] = _pack(c)
                return put

            arrive(0)
            zero_s[...] = jnp.zeros(zero_s.shape, U32)
            gw_b[:, :, h:h + 2 * HALO, :] = jnp.zeros((2, NL, 2 * HALO, 128), F32)
            stage(0, _dot, wao_s, lambda: wm_s[0:D, :], put_plain)
            arrive(1)
            stage(1, _dot, wv_s, lambda: t_s[...], put_rhs(oc_s, 0))
            arrive(2)
            stage(2, _dot_nt, wq_s, lambda: wk_s[...], put_rhs(mc_s, 0, float(D) ** -0.5 * math.log2(math.e)))
            arrive(3)
            stage(3, _dot, wdn_s, lambda: wm_s[D:2 * D, :], put_rhs(oc_s, D2))
            arrive(4)
            x_copy(1, 0, T2, 4).start()
            for r in range(0, D2, 64):
                w = jnp.concatenate([wup_s[r:r + 64, 0:D], wup_s[D2 + r:D2 + r + 64, 0:D]], axis=0)
                put_rhs(uc_s, 0)(r, 64, w.astype(F32))
            wg_s[...] = pltpu.bitcast(wup_s[:, D:2 * D], U32)
            dwf = dw_s[...].astype(F32)
            for k in range(K):
                dwb_s[k] = jnp.broadcast_to(dwf[k:k + 1, :], (8, D))
            edges(0)

        @pl.when(step == 1)
        def _():
            x_copy(1, 0, T2, 4).wait()

        @pl.when(step == first)
        def _():
            edges(1)

        slot = step % 2
        spare8 = pl.multiple_of(8 * (2 * step // nt), 8)
        clock = [0]
        due = []

        def release(work, n, slots, val):
            todo = work[n * len(work) // slots:(n + 1) * len(work) // slots] if n < slots else []
            for k, piece in enumerate(todo):
                r = (h * k // len(todo)) // 8 * 8
                due.append((clock[0] + DLY, piece(val[r:r + 8, 0:128])))

        def mm(dot, lhs, w):
            bits = None
            due.sort(key=lambda e: e[0])
            while due and due[0][0] <= clock[0]:
                tok = pltpu.bitcast(due.pop(0)[1], U32)
                for a in range(0, tok.shape[0], 8):
                    bits = tok[a:a + 8] if bits is None else bits | tok[a:a + 8]
            if bits is not None:
                head = jnp.concatenate([w[0:8, 0:128] | (bits & zero_s[...]), w[0:8, 128:]], axis=1)
                w = jnp.concatenate([head, w[8:]], axis=0)
            r = dot(lhs, _unpack(w))
            due.append((clock[0] + ORD, r[0:8, 0:128]))
            clock[0] += 1
            return r

        class Tile:
            def __init__(self, t, gw, gw_prev, z, s):
                self.b = t // nt
                self.i = t % nt
                self.r0 = pl.multiple_of(self.i * h, 16)
                self.gw, self.gw_prev, self.z, self.s = gw, gw_prev, z, s
                self.lsum, self.lse, self.pc, self.zc = {}, {}, {}, {}

            def xc(self, i, off):
                rows = pl.ds(pl.multiple_of(self.i * (h // 2) + off // 2, 8), h // 2)
                return xc_s[self.b, i, rows, :]

            def proj(self, w_ref):
                return _seven(lambda i: mm(_dot, _unpack(self.xc(i, 0)), w_ref[i]))

            def proj_g(self):
                xg = jnp.concatenate([
                    jnp.concatenate([self.xc(2, HALO), self.xc(7, HALO)], axis=1),
                    jnp.concatenate([self.xc(8, HALO), self.xc(3, HALO)], axis=1)], axis=0)
                g = _ln(_gelu(_dot(_unpack(xg), _unpack(wg_s[...]))))
                for hf in range(2):
                    for j in range(NL):
                        self.gw[hf, j, 0:2 * HALO, :] = jnp.where(
                            self.i == 0, gi_s[self.b, hf, j], self.gw_prev[hf, j, h:h + 2 * HALO, :])
                        self.gw[hf, j, 2 * HALO:h + 2 * HALO, :] = g[hf * h:(hf + 1) * h, j * 128:(j + 1) * 128]

            def proj_u(self):
                c11, c12, c21, c22 = self.proj(uc_s)
                for hf, (lo, hi) in enumerate(((c11, c12), (c21, c22))):
                    for n in range(2):
                        self.z[hf, n, 0:h, :] = _gelu(lo[:, n * 128:(n + 1) * 128])
                        self.z[hf, 2 + n, 0:h, :] = _gelu(hi[:, n * 128:(n + 1) * 128])

            def proj_q(self):
                q11, q12, q21, q22 = self.proj(mc_s)
                self.qc = [c.astype(BF16) for c in
                           (q11 + q22, q21 + q22, q11, q22, q11 + q12, q21 - q11, q12 - q22)]

            def conv_piece(self, hf, j, a, gate):
                self.gw[hf, j, pl.ds(h + 2 * HALO + spare8, 8), :] = gate
                acc = None
                for k in sorted(range(K), key=lambda k: (k % 8, k)):
                    w = dwb_s[k, :, j * 128:(j + 1) * 128]
                    t = self.gw[hf, j, a + k + 1:a + k + 17, :].reshape(2, 8, 128) * w[None]
                    acc = t if acc is None else acc + t
                z = acc.reshape(16, 128) * self.z[hf, j, a:a + 16, :]
                self.z[hf, j, a:a + 16, :] = z
                return z

            def z_piece(self, a, gate):
                self.z[0, 0, pl.ds(h + spare8, 8), :] = gate
                tiles = [_lhs_combos(*[self.z[hf, 2 * s + n, a:a + 16, :] for hf in range(2) for s in range(2)])
                         for n in range(2)]
                self.zc[a] = [jnp.concatenate([t[i] for t in tiles], axis=1) for i in range(7)]
                return tiles[1][6]

            def conv_pieces(self):
                work = []
                for a in range(0, h, 16):
                    work += [lambda g, hf=hf, j=j, a=a: self.conv_piece(hf, j, a, g)
                             for hf in range(2) for j in range(NL)]
                    work.append(lambda g, a=a: self.z_piece(a, g))
                return work

            def logits(self, work, margin):
                nchunk = TP // QC
                src = (0, 2, 1, 4, 3, 5, 6)
                mx = [None, None]
                done = []
                for c in range(nchunk):
                    keys = pl.ds(c * QC // 2, QC // 2)

                    def prod(i):
                        r = mm(_dot_nt, self.qc[i], xc_s[self.b, src[i], keys, :])
                        release(work, len(done), nchunk * 7 - margin, r)
                        done.append(True)
                        return r

                    def emit(hf, side, val):
                        for n in range(QC // 128):
                            kt = c * (QC // 128) + n
                            t = val[:, n * 128:(n + 1) * 128]
                            if (kt + 1) * 128 > T2:
                                col = kt * 128 + lax.broadcasted_iota(jnp.int32, (h, 128), 1)
                                t = jnp.where(col < T2, t, -jnp.inf)
                            self.s[hf, side, kt, 0:h, :] = t
                            mx[hf] = t if mx[hf] is None else jnp.maximum(mx[hf], t)

                    t11 = prod(6)
                    m4 = prod(3)
                    t11 = t11 - m4
                    m2 = prod(1)
                    emit(1, 0, m2 - m4)
                    m1 = prod(0)
                    t11 = t11 + m1
                    t22 = m1 - m2
                    m5 = prod(4)
                    emit(0, 0, t11 - m5)
                    m3 = prod(2)
                    emit(0, 1, m5 - m3)
                    emit(1, 1, (t22 - m3) + prod(5))
                self.m = [jnp.max(v, axis=-1, keepdims=True) for v in mx]

            def gate_s(self, gate):
                self.s[0, 0, 0, pl.ds(h + spare8, 8), :] = gate

            def sum_piece(self, hf, a, tiles, last, gate):
                self.gate_s(gate)
                m = self.m[hf][a:a + 16]
                mb = jnp.broadcast_to(m, (16, 128))
                acc = self.lsum.get((hf, a))
                for side, kt in tiles:
                    e = jnp.exp2(self.s[hf, side, kt, a:a + 16, :] - mb)
                    acc = e if acc is None else acc + e
                self.lsum[hf, a] = acc
                if last:
                    l = jnp.sum(acc, axis=-1, keepdims=True)
                    acc = self.lse[hf, a] = jnp.broadcast_to(m + jnp.log2(l), (16, 128))
                return acc

            def sum_pieces(self):
                tiles = [(side, kt) for side in range(2) for kt in range(NKT)]
                work = []
                for a in range(0, h, 16):
                    work += [lambda g, hf=hf, a=a, n=n: self.sum_piece(hf, a, tiles[n:n + SUMT], n + SUMT >= len(tiles), g)
                             for hf in range(2) for n in range(0, len(tiles), SUMT)]
                    work += [lambda g, kt=kt, a=a: self.exp_piece(kt, a, g) for kt in range(0, PC // 128, EXPT)]
                return work

            def exp_piece(self, kt0, a, gate):
                self.gate_s(gate)
                tok = None
                for kt in range(kt0, kt0 + EXPT):
                    p = [jnp.exp2(self.s[hf, side, kt, a:a + 16, :] - self.lse[hf, a])
                         for hf in range(2) for side in range(2)]
                    cs = self.pc[kt, a] = _lhs_combos(*p)
                    t = cs[5] + cs[6]
                    tok = t if tok is None else tok + t
                return tok

            def exp_pieces(self, c):
                return [lambda g, kt=kt, a=a: self.exp_piece(kt, a, g)
                        for a in range(0, h, 16) for kt in range(c * PC // 128, (c + 1) * PC // 128, EXPT)]

            def attend(self, extra):
                src = (0, 2, 6, 5, 3, 4, 1)
                acc = [None] * 7
                for c in range(npv):
                    keys = pl.ds(c * PC // 2, PC // 2)
                    work = _mix(self.exp_pieces(c + 1) if c + 1 < npv else [], *[e[c] for e in extra])
                    for n, i in enumerate((1, 3, 0, 6, 4, 2, 5)):
                        p = jnp.concatenate([
                            jnp.concatenate([self.pc[kt, a][i] for kt in range(c * PC // 128, (c + 1) * PC // 128)], axis=1)
                            for a in range(0, h, 16)], axis=0).astype(BF16)
                        r = mm(_dot, p, xc_s[self.b, src[i], keys, :])
                        acc[i] = r if acc[i] is None else acc[i] + r
                        release(work, n, 7 - PV_MARGIN, acc[i])
                n1, n2, n3, n4, n5, n6, n7 = acc
                self.oc = _lhs_combos(n1 - n4 - n5 - n7, n3 - n5, n4 - n2, n1 - n2 - n3 - n6)

            def out(self, dst):
                zc = [jnp.concatenate([self.zc[a][i] for a in range(0, h, 16)], axis=0) for i in range(7)]
                c11, c12, c21, c22 = _seven(
                    lambda i: mm(_dot, jnp.concatenate([self.oc[i], zc[i]], axis=1).astype(BF16), oc_s[i]))
                for hf, (lo, hi) in enumerate(((c11, c12), (c21, c22))):
                    res = x_s[self.b, hf, pl.ds(self.r0, h), :].astype(F32)
                    o_s[slot, dst, hf] = (jnp.concatenate([lo, hi], axis=1) + res).astype(o_s.dtype)

            def out_copy(self, sl, dst):
                return pltpu.make_async_copy(
                    o_s.at[sl, dst], o_hbm.at[self.b, :, pl.ds(self.r0, h), :], osem.at[sl, dst])

        def fill_piece(n, gate):
            r = jnp.clip((step - 1) * fill_rows + n * 16, 0, T2 - 16)
            rows = pl.ds(pl.multiple_of(r, 16), 16)
            bb = jnp.minimum(step, 1)
            hold = pltpu.bitcast(gate, U32) & zero_s[...]
            top, bot = [_unpack(pltpu.bitcast(x_s[bb, hf, rows, :], U32) | jnp.concatenate([hold] * NL, axis=1))
                        for hf in range(2)]
            cs = ln_rows(top, bot)
            for i, c in enumerate(cs):
                st_s[i, n * 8:n * 8 + 8, :] = c
            return cs[0][:, 0:128]

        def fill_store(rows):
            dst = pl.ds(pl.multiple_of((step - 1) * (fill_rows // 2), 8), rows // 2)
            for i in range(9):
                xc_s[1, i, dst, :] = st_s[i, 0:rows // 2, :]

        ta = Tile(2 * step, gw_a, gw_b, z_a, s_a)
        tb = Tile(2 * step + 1, gw_b, gw_a, z_b, s_b)

        @pl.when(step >= 2)
        def _():
            ta.out_copy(slot, 0).wait()
            tb.out_copy(slot, 1).wait()

        conv = _share(ta.conv_pieces() + tb.conv_pieces(), SPLIT)
        fills = [lambda g, n=n: fill_piece(n, g) for n in range(fill_rows // 16)]
        for t in (ta, tb):
            t.proj_g()
            t.proj_q()
        ta.proj_u()
        tb.proj_u()
        ta.logits(conv[0], 0)
        tb.logits(_mix(conv[1], ta.sum_pieces()), QK_MARGIN)
        ta.attend([_share(tb.sum_pieces(), SUM_B), _share(conv[2], (1,) * npv)])
        tb.attend([_share(conv[3], (0,) * (npv - 1) + (1,)), _share(fills, (1,) * (npv - 1) + (0,))])
        ta.out(0)
        tb.out(1)
        ta.out_copy(slot, 0).start()
        tb.out_copy(slot, 1).start()

        @pl.when((step >= 1) & (step < nfill))
        def _():
            fill_store(fill_rows)

        @pl.when(step == nfill)
        def _():
            fill_store(last_rows)

        @pl.when(step == nsteps - 1)
        def _():
            for sl in (slot, 1 - slot):
                ta.out_copy(sl, 0).wait()
                tb.out_copy(sl, 1).wait()

    vmem = pltpu.VMEM
    gw_shape = (2, NL, h + 2 * HALO + 16, 128)
    z_shape = (2, NL, h + 16, 128)
    s_shape = (2, 2, NKT, h + 16, 128)
    out = pl.pallas_call(
        kernel,
        grid=(B * nt // 2,),
        in_specs=[pl.BlockSpec(memory_space=pl.ANY)] * 9,
        out_specs=pl.BlockSpec(memory_space=pl.ANY),
        out_shape=jax.ShapeDtypeStruct((B, 2, T2, D), x.dtype),
        scratch_shapes=[
            vmem((B, 2, T2, D), BF16),
            vmem((D, D), BF16), vmem((D, D), BF16), vmem((D, D), BF16), vmem((D, D), BF16),
            vmem((D, 2 * D), BF16), vmem((K, D), BF16), vmem((D, D), BF16), vmem((2 * D, D), BF16),
            pltpu.SemaphoreType.DMA((9,)), pltpu.SemaphoreType.DMA((5,)), pltpu.SemaphoreType.DMA((2, 2)),
            vmem((7, D2 // 2, D2), U32), vmem((7, D2 // 2, D2), U32), vmem((7, D2, D2), U32),
            vmem((K, 8, D), F32),
            vmem((B, 9, TP // 2, D2), U32),
            vmem((B, 2, NL, 2 * HALO, 128), F32),
            vmem((2, 2, 2, h, D), x.dtype),
            vmem(gw_shape, F32), vmem(gw_shape, F32),
            vmem(z_shape, F32), vmem(z_shape, F32),
            vmem(s_shape, F32), vmem(s_shape, F32),
            vmem((8, 128), U32),
            vmem((9, fill_rows // 2, D2), U32),
            vmem((D, D), BF16), vmem((D2, D), U32),
        ],
        compiler_params=pltpu.CompilerParams(
            dimension_semantics=("arbitrary",),
            vmem_limit_bytes=100 * 1024 * 1024,
            disable_bounds_checks=True,
        ),
    )(x.reshape(B, 2, T2, D), w_q, w_k, w_v, w_ao, w_up, dw, w_dn, w_merge)
    return out.reshape(B, T, D)
```

```python
import math

import jax
import jax.experimental.pallas as pl
import jax.experimental.pallas.tpu as pltpu
import jax.numpy as jnp
import numpy as np
from jax import lax

F32 = jnp.float32
BF16 = jnp.bfloat16
U32 = jnp.uint32

H = 80
QC = 256
PC = 512
HALO = 16
EPS = 1e-5

DLY = 6
ORD = 3
SUMT = 8
EXPT = 2
SPLIT = (55, 15, 5, 15)
SUM_B = (1, 1, 1, 2)
QK_MARGIN = 6
PV_MARGIN = 1


def _dot(a, b):
    return jnp.dot(a, b, preferred_element_type=F32)


def _dot_nt(a, b):
    return lax.dot_general(a, b, (((1,), (1,)), ((), ())), preferred_element_type=F32)


def _pack(v):
    return pltpu.bitcast(v.astype(BF16), U32)


def _unpack(w):
    return pltpu.bitcast(w, BF16)


def _ln(x):
    m = jnp.mean(x, axis=-1, keepdims=True)
    xc = x - m
    v = jnp.mean(xc * xc, axis=-1, keepdims=True)
    return xc * lax.rsqrt(v + EPS)


def _gelu(x):
    c = math.sqrt(2.0 / math.pi)
    hx = 0.5 * x
    return hx + hx * jnp.tanh(x * (c + (c * 0.044715) * (x * x)))


def _lhs_combos(a11, a12, a21, a22):
    return (a11 + a22, a22 - a21, a11, a22, a11 - a12, a21 + a11, a12 + a22)


def _rhs_combos(b11, b12, b21, b22):
    return (b11 + b22, b11, b12 + b22, b21 + b11, b22, b12 - b11, b21 - b22)


def _quads(w):
    r, c = w.shape[0] // 2, w.shape[1] // 2
    return w[:r, :c], w[:r, c:], w[r:, :c], w[r:, c:]


def _seven(prod):
    n2 = prod(1)
    n4 = prod(3)
    c21 = n4 - n2
    n1 = prod(0)
    t11 = n1 - n4
    t22 = n1 - n2
    t11 = t11 + prod(6)
    n5 = prod(4)
    c11 = t11 - n5
    n3 = prod(2)
    c12 = n3 - n5
    c22 = (t22 - n3) + prod(5)
    return c11, c12, c21, c22


def _mix(*lists):
    keyed = [((n + 0.5) / len(l), k, n, w) for k, l in enumerate(lists) for n, w in enumerate(l)]
    return [e[3] for e in sorted(keyed, key=lambda e: e[:3])]


def _share(items, weights):
    cut = [len(items) * int(n) // sum(weights) for n in np.cumsum((0,) + tuple(weights))]
    return [items[a:b] for a, b in zip(cut, cut[1:])]


@jax.jit
def pallas_standalone__conformer_family_branchformer__speech_kernel(
    x: jax.Array,
    w_q: jax.Array,
    w_k: jax.Array,
    w_v: jax.Array,
    w_ao: jax.Array,
    w_up: jax.Array,
    dw: jax.Array,
    w_dn: jax.Array,
    w_merge: jax.Array,
):
    B, T, D = x.shape
    K = dw.shape[0]
    T2 = T // 2
    D2 = D // 2
    NL = D // 128
    h = H
    nt = T2 // h
    TP = -(-T2 // PC) * PC
    NKT = TP // 128
    npv = TP // PC
    first = nt // 2
    nfill = first - 1
    fill_rows = -(-(T2 // 16) // nfill) * 16
    last_rows = T2 - (nfill - 1) * fill_rows
    assert B == 2 and nt <= 32 and T2 % h == 0 and TP >= T2 + HALO and K == 2 * HALO - 1 and last_rows > 0

    def kernel(x_hbm, wq_hbm, wk_hbm, wv_hbm, wao_hbm, wup_hbm, dw_hbm, wdn_hbm, wm_hbm, o_hbm,
               x_s, wq_s, wk_s, wv_s, wao_s, wup_s, dw_s, wdn_s, wm_s, wsem, xsem, osem,
               mc_s, uc_s, oc_s, dwb_s, xc_s, gi_s, o_s,
               gw_a, gw_b, z_a, z_b, s_a, s_b, zero_s, st_s, t_s, wg_s):
        step = pl.program_id(0)
        nsteps = pl.num_programs(0)

        def ln_rows(top, bot):
            t, b = _ln(top.astype(F32)), _ln(bot.astype(F32))
            x11, x12, x21, x22 = t[:, :D2], t[:, D2:], b[:, :D2], b[:, D2:]
            return [_pack(c) for c in _lhs_combos(x11, x12, x21, x22) + (x12, x21)]

        def edges(bb):
            over = x_s[bb, 1, 0:HALO, :]
            for i, c in enumerate(ln_rows(over, jnp.zeros((HALO, D), BF16))):
                xc_s[bb, i, T2 // 2:(T2 + HALO) // 2, :] = c
            xc_s[bb, :, (T2 + HALO) // 2:, :] = jnp.zeros((9, (TP - T2 - HALO) // 2, D2), U32)
            xe = jnp.concatenate([x_s[bb, 0, 0:HALO, :], x_s[bb, 0, T2 - HALO:T2, :], over], axis=0)
            ge = _ln(_gelu(_dot(_ln(xe.astype(F32)).astype(BF16), wup_s[:, D:2 * D])))
            for j in range(NL):
                gi_s[bb, 0, j, 0:HALO, :] = jnp.zeros((HALO, 128), F32)
                gi_s[bb, 0, j, HALO:, :] = ge[0:HALO, j * 128:(j + 1) * 128]
                gi_s[bb, 1, j, :, :] = ge[HALO:, j * 128:(j + 1) * 128]

        def x_copy(bb, r0, r1, n):
            rows = (bb, slice(None), pl.ds(r0, r1 - r0))
            return pltpu.make_async_copy(x_hbm.at[rows], x_s.at[rows], xsem.at[n])

        @pl.when(step == 0)
        def _():
            top, bot = pl.ds(0, D), pl.ds(D, D)
            cp = [pltpu.make_async_copy(s, d, wsem.at[n]) for n, (s, d) in enumerate([
                (wao_hbm, wao_s), (wm_hbm.at[top], wm_s.at[top]), (wv_hbm, wv_s),
                (wq_hbm, wq_s), (wk_hbm, wk_s), (wdn_hbm, wdn_s), (wm_hbm.at[bot], wm_s.at[bot]),
                (dw_hbm, dw_s), (wup_hbm, wup_s)])]
            cuts = [T2 // 16 * n // 4 * 16 for n in range(5)]
            xp = [x_copy(0, cuts[n], cuts[n + 1], n) for n in range(4)]
            stages = [[cp[0], cp[1], xp[0]], [cp[2], xp[1]], [cp[3], cp[4], xp[2]], [cp[5], cp[6], xp[3]],
                      [cp[7], cp[8], x_copy(1, 0, HALO, 5), x_copy(1, T2 - HALO, T2, 6)]]
            started = []

            def arrive(n):
                while len(started) < min(n + 3, len(stages)):
                    for c in stages[len(started)]:
                        c.start()
                    started.append(True)
                for c in stages[n]:
                    c.wait()

            def stage(n, dot, lhs_ref, rhs, put):
                sub = [cuts[n] + (cuts[n + 1] - cuts[n]) // 16 * k // 12 * 16 for k in range(13)]
                wr = D2 // 2
                for k in range(2):
                    lhs = jnp.concatenate([lhs_ref[k * wr:(k + 1) * wr, :],
                                           lhs_ref[D2 + k * wr:D2 + (k + 1) * wr, :]], axis=0)
                    put(k * wr, wr, dot(lhs, rhs()))
                    for r0, r1 in zip(sub[k * 6:(k + 1) * 6], sub[k * 6 + 1:]):
                        for i, c in enumerate(ln_rows(x_s[0, 0, r0:r1, :], x_s[0, 1, r0:r1, :])):
                            xc_s[0, i, r0 // 2:r1 // 2, :] = c

            def put_plain(r, n, w):
                t_s[r:r + n, :] = w[:n].astype(BF16)
                t_s[D2 + r:D2 + r + n, :] = w[n:].astype(BF16)

            def put_rhs(dst, k0, scale=None):
                def put(r, n, w):
                    if scale is not None:
                        w = w * scale
                    for i, c in enumerate(_rhs_combos(*_quads(w))):
                        dst[i, (k0 + r) // 2:(k0 + r + n) // 2, :] = _pack(c)
                return put

            arrive(0)
            zero_s[...] = jnp.zeros(zero_s.shape, U32)
            gw_b[:, :, h:h + 2 * HALO, :] = jnp.zeros((2, NL, 2 * HALO, 128), F32)
            stage(0, _dot, wao_s, lambda: wm_s[0:D, :], put_plain)
            arrive(1)
            stage(1, _dot, wv_s, lambda: t_s[...], put_rhs(oc_s, 0))
            arrive(2)
            stage(2, _dot_nt, wq_s, lambda: wk_s[...], put_rhs(mc_s, 0, float(D) ** -0.5 * math.log2(math.e)))
            arrive(3)
            stage(3, _dot, wdn_s, lambda: wm_s[D:2 * D, :], put_rhs(oc_s, D2))
            arrive(4)
            edges(1)
            x_copy(1, 0, T2, 4).start()
            for r in range(0, D2, 64):
                w = jnp.concatenate([wup_s[r:r + 64, 0:D], wup_s[D2 + r:D2 + r + 64, 0:D]], axis=0)
                put_rhs(uc_s, 0)(r, 64, w.astype(F32))
            wg_s[...] = pltpu.bitcast(wup_s[:, D:2 * D], U32)
            dwf = dw_s[...].astype(F32)
            for k in range(K):
                dwb_s[k] = jnp.broadcast_to(dwf[k:k + 1, :], (8, D))
            edges(0)

        @pl.when(step == 1)
        def _():
            x_copy(1, 0, T2, 4).wait()

        slot = step % 2
        spare8 = pl.multiple_of(8 * (step >> 4), 8)
        clock = [0]
        due = []

        def release(work, n, slots, val):
            todo = work[n * len(work) // slots:(n + 1) * len(work) // slots] if n < slots else []
            for k, piece in enumerate(todo):
                r = (h * k // len(todo)) // 8 * 8
                due.append((clock[0] + DLY, piece(val[r:r + 8, 0:128])))

        def mm(dot, lhs, w):
            bits = None
            due.sort(key=lambda e: e[0])
            while due and due[0][0] <= clock[0]:
                tok = pltpu.bitcast(due.pop(0)[1], U32)
                for a in range(0, tok.shape[0], 8):
                    bits = tok[a:a + 8] if bits is None else bits | tok[a:a + 8]
            if bits is not None:
                head = jnp.concatenate([w[0:8, 0:128] | (bits & zero_s[...]), w[0:8, 128:]], axis=1)
                w = jnp.concatenate([head, w[8:]], axis=0)
            r = dot(lhs, _unpack(w))
            due.append((clock[0] + ORD, r[0:8, 0:128]))
            clock[0] += 1
            return r

        class Tile:
            def __init__(self, t, gw, gw_prev, z, s):
                self.b = (t >= nt).astype(jnp.int32)
                self.i = t - self.b * nt
                self.r0 = pl.multiple_of(self.i * h, 16)
                self.gw, self.gw_prev, self.z, self.s = gw, gw_prev, z, s
                self.lsum, self.lse, self.pc, self.zc = {}, {}, {}, {}

            def xc(self, i, off):
                rows = pl.ds(pl.multiple_of(self.i * (h // 2) + off // 2, 8), h // 2)
                return xc_s[self.b, i, rows, :]

            def proj(self, w_ref):
                return _seven(lambda i: mm(_dot, _unpack(self.xc(i, 0)), w_ref[i]))

            def proj_g(self):
                xg = jnp.concatenate([
                    jnp.concatenate([self.xc(2, HALO), self.xc(7, HALO)], axis=1),
                    jnp.concatenate([self.xc(8, HALO), self.xc(3, HALO)], axis=1)], axis=0)
                g = _ln(_gelu(_dot(_unpack(xg), _unpack(wg_s[...]))))
                for hf in range(2):
                    for j in range(NL):
                        self.gw[hf, j, 0:2 * HALO, :] = jnp.where(
                            self.i == 0, gi_s[self.b, hf, j], self.gw_prev[hf, j, h:h + 2 * HALO, :])
                        self.gw[hf, j, 2 * HALO:h + 2 * HALO, :] = g[hf * h:(hf + 1) * h, j * 128:(j + 1) * 128]

            def proj_u(self):
                c11, c12, c21, c22 = self.proj(uc_s)
                for hf, (lo, hi) in enumerate(((c11, c12), (c21, c22))):
                    for n in range(2):
                        self.z[hf, n, 0:h, :] = _gelu(lo[:, n * 128:(n + 1) * 128])
                        self.z[hf, 2 + n, 0:h, :] = _gelu(hi[:, n * 128:(n + 1) * 128])

            def proj_q(self):
                q11, q12, q21, q22 = self.proj(mc_s)
                self.qc = [c.astype(BF16) for c in
                           (q11 + q22, q21 + q22, q11, q22, q11 + q12, q21 - q11, q12 - q22)]

            def conv_piece(self, hf, j, a, gate):
                self.gw[hf, j, pl.ds(h + 2 * HALO + spare8, 8), :] = gate
                acc = None
                for k in sorted(range(K), key=lambda k: (k % 8, k)):
                    w = dwb_s[k, :, j * 128:(j + 1) * 128]
                    t = self.gw[hf, j, a + k + 1:a + k + 17, :].reshape(2, 8, 128) * w[None]
                    acc = t if acc is None else acc + t
                z = acc.reshape(16, 128) * self.z[hf, j, a:a + 16, :]
                self.z[hf, j, a:a + 16, :] = z
                return z

            def z_piece(self, a, gate):
                self.z[0, 0, pl.ds(h + spare8, 8), :] = gate
                tiles = [_lhs_combos(*[self.z[hf, 2 * s + n, a:a + 16, :] for hf in range(2) for s in range(2)])
                         for n in range(2)]
                self.zc[a] = [jnp.concatenate([t[i] for t in tiles], axis=1) for i in range(7)]
                return tiles[1][6]

            def conv_pieces(self):
                work = []
                for a in range(0, h, 16):
                    work += [lambda g, hf=hf, j=j, a=a: self.conv_piece(hf, j, a, g)
                             for hf in range(2) for j in range(NL)]
                    work.append(lambda g, a=a: self.z_piece(a, g))
                return work

            def logits(self, work, margin):
                nchunk = TP // QC
                src = (0, 2, 1, 4, 3, 5, 6)
                mx = [None, None]
                done = []
                for c in range(nchunk):
                    keys = pl.ds(c * QC // 2, QC // 2)

                    def prod(i):
                        r = mm(_dot_nt, self.qc[i], xc_s[self.b, src[i], keys, :])
                        release(work, len(done), nchunk * 7 - margin, r)
                        done.append(True)
                        return r

                    def emit(hf, side, val):
                        for n in range(QC // 128):
                            kt = c * (QC // 128) + n
                            t = val[:, n * 128:(n + 1) * 128]
                            if (kt + 1) * 128 > T2:
                                col = kt * 128 + lax.broadcasted_iota(jnp.int32, (h, 128), 1)
                                t = jnp.where(col < T2, t, -jnp.inf)
                            self.s[hf, side, kt, 0:h, :] = t
                            mx[hf] = t if mx[hf] is None else jnp.maximum(mx[hf], t)

                    t11 = prod(6)
                    m4 = prod(3)
                    t11 = t11 - m4
                    m2 = prod(1)
                    emit(1, 0, m2 - m4)
                    m1 = prod(0)
                    t11 = t11 + m1
                    t22 = m1 - m2
                    m5 = prod(4)
                    emit(0, 0, t11 - m5)
                    m3 = prod(2)
                    emit(0, 1, m5 - m3)
                    emit(1, 1, (t22 - m3) + prod(5))
                self.m = [jnp.max(v, axis=-1, keepdims=True) for v in mx]

            def gate_s(self, gate):
                self.s[0, 0, 0, pl.ds(h + spare8, 8), :] = gate

            def sum_piece(self, hf, a, tiles, last, gate):
                self.gate_s(gate)
                m = self.m[hf][a:a + 16]
                mb = jnp.broadcast_to(m, (16, 128))
                acc = self.lsum.get((hf, a))
                for side, kt in tiles:
                    e = jnp.exp2(self.s[hf, side, kt, a:a + 16, :] - mb)
                    acc = e if acc is None else acc + e
                self.lsum[hf, a] = acc
                if last:
                    l = jnp.sum(acc, axis=-1, keepdims=True)
                    acc = self.lse[hf, a] = jnp.broadcast_to(m + jnp.log2(l), (16, 128))
                return acc

            def sum_pieces(self):
                tiles = [(side, kt) for side in range(2) for kt in range(NKT)]
                work = []
                for a in range(0, h, 16):
                    work += [lambda g, hf=hf, a=a, n=n: self.sum_piece(hf, a, tiles[n:n + SUMT], n + SUMT >= len(tiles), g)
                             for hf in range(2) for n in range(0, len(tiles), SUMT)]
                    work += [lambda g, kt=kt, a=a: self.exp_piece(kt, a, g) for kt in range(0, PC // 128, EXPT)]
                return work

            def exp_piece(self, kt0, a, gate):
                self.gate_s(gate)
                tok = None
                for kt in range(kt0, kt0 + EXPT):
                    p = [jnp.exp2(self.s[hf, side, kt, a:a + 16, :] - self.lse[hf, a])
                         for hf in range(2) for side in range(2)]
                    cs = self.pc[kt, a] = _lhs_combos(*p)
                    t = cs[5] + cs[6]
                    tok = t if tok is None else tok + t
                return tok

            def exp_pieces(self, c):
                return [lambda g, kt=kt, a=a: self.exp_piece(kt, a, g)
                        for a in range(0, h, 16) for kt in range(c * PC // 128, (c + 1) * PC // 128, EXPT)]

            def attend(self, extra):
                src = (0, 2, 6, 5, 3, 4, 1)
                acc = [None] * 7
                for c in range(npv):
                    keys = pl.ds(c * PC // 2, PC // 2)
                    work = _mix(self.exp_pieces(c + 1) if c + 1 < npv else [], *[e[c] for e in extra])
                    for n, i in enumerate((1, 3, 0, 6, 4, 2, 5)):
                        p = jnp.concatenate([
                            jnp.concatenate([self.pc[kt, a][i] for kt in range(c * PC // 128, (c + 1) * PC // 128)], axis=1)
                            for a in range(0, h, 16)], axis=0).astype(BF16)
                        r = mm(_dot, p, xc_s[self.b, src[i], keys, :])
                        acc[i] = r if acc[i] is None else acc[i] + r
                        release(work, n, 7 - PV_MARGIN, acc[i])
                n1, n2, n3, n4, n5, n6, n7 = acc
                self.oc = _lhs_combos(n1 - n4 - n5 - n7, n3 - n5, n4 - n2, n1 - n2 - n3 - n6)

            def out(self, dst):
                zc = [jnp.concatenate([self.zc[a][i] for a in range(0, h, 16)], axis=0) for i in range(7)]
                c11, c12, c21, c22 = _seven(
                    lambda i: mm(_dot, jnp.concatenate([self.oc[i], zc[i]], axis=1).astype(BF16), oc_s[i]))
                for hf, (lo, hi) in enumerate(((c11, c12), (c21, c22))):
                    res = x_s[self.b, hf, pl.ds(self.r0, h), :].astype(F32)
                    o_s[slot, dst, hf] = (jnp.concatenate([lo, hi], axis=1) + res).astype(o_s.dtype)

            def out_copy(self, sl, dst):
                return pltpu.make_async_copy(
                    o_s.at[sl, dst], o_hbm.at[self.b, :, pl.ds(self.r0, h), :], osem.at[sl, dst])

        def fill_piece(n, gate):
            r = jnp.clip((step - 1) * fill_rows + n * 16, 0, T2 - 16)
            rows = pl.ds(pl.multiple_of(r, 16), 16)
            bb = jnp.minimum(step, 1)
            hold = pltpu.bitcast(gate, U32) & zero_s[...]
            top, bot = [_unpack(pltpu.bitcast(x_s[bb, hf, rows, :], U32) | jnp.concatenate([hold] * NL, axis=1))
                        for hf in range(2)]
            cs = ln_rows(top, bot)
            for i, c in enumerate(cs):
                st_s[i, n * 8:n * 8 + 8, :] = c
            return cs[0][:, 0:128]

        def fill_store(rows):
            dst = pl.ds(pl.multiple_of((step - 1) * (fill_rows // 2), 8), rows // 2)
            for i in range(9):
                xc_s[1, i, dst, :] = st_s[i, 0:rows // 2, :]

        ta = Tile(2 * step, gw_a, gw_b, z_a, s_a)
        tb = Tile(2 * step + 1, gw_b, gw_a, z_b, s_b)

        @pl.when(step >= 2)
        def _():
            ta.out_copy(slot, 0).wait()
            tb.out_copy(slot, 1).wait()

        conv = _share(ta.conv_pieces() + tb.conv_pieces(), SPLIT)
        fills = [lambda g, n=n: fill_piece(n, g) for n in range(fill_rows // 16)]
        for t in (ta, tb):
            t.proj_g()
            t.proj_q()
        ta.proj_u()
        tb.proj_u()
        ta.logits(conv[0], 0)
        tb.logits(_mix(conv[1], ta.sum_pieces()), QK_MARGIN)
        ta.attend([_share(tb.sum_pieces(), SUM_B), _share(conv[2], (1,) * npv)])
        tb.attend([_share(conv[3], (0,) * (npv - 1) + (1,)), _share(fills, (1,) * (npv - 1) + (0,))])
        ta.out(0)
        tb.out(1)
        ta.out_copy(slot, 0).start()
        tb.out_copy(slot, 1).start()

        @pl.when((step >= 1) & (step < nfill))
        def _():
            fill_store(fill_rows)

        @pl.when(step == nfill)
        def _():
            fill_store(last_rows)

        @pl.when(step == nsteps - 1)
        def _():
            for sl in (slot, 1 - slot):
                ta.out_copy(sl, 0).wait()
                tb.out_copy(sl, 1).wait()

    vmem = pltpu.VMEM
    gw_shape = (2, NL, h + 2 * HALO + 16, 128)
    z_shape = (2, NL, h + 16, 128)
    s_shape = (2, 2, NKT, h + 16, 128)
    out = pl.pallas_call(
        kernel,
        grid=(B * nt // 2,),
        in_specs=[pl.BlockSpec(memory_space=pl.ANY)] * 9,
        out_specs=pl.BlockSpec(memory_space=pl.ANY),
        out_shape=jax.ShapeDtypeStruct((B, 2, T2, D), x.dtype),
        scratch_shapes=[
            vmem((B, 2, T2, D), BF16),
            vmem((D, D), BF16), vmem((D, D), BF16), vmem((D, D), BF16), vmem((D, D), BF16),
            vmem((D, 2 * D), BF16), vmem((K, D), BF16), vmem((D, D), BF16), vmem((2 * D, D), BF16),
            pltpu.SemaphoreType.DMA((9,)), pltpu.SemaphoreType.DMA((7,)), pltpu.SemaphoreType.DMA((2, 2)),
            vmem((7, D2 // 2, D2), U32), vmem((7, D2 // 2, D2), U32), vmem((7, D2, D2), U32),
            vmem((K, 8, D), F32),
            vmem((B, 9, TP // 2, D2), U32),
            vmem((B, 2, NL, 2 * HALO, 128), F32),
            vmem((2, 2, 2, h, D), x.dtype),
            vmem(gw_shape, F32), vmem(gw_shape, F32),
            vmem(z_shape, F32), vmem(z_shape, F32),
            vmem(s_shape, F32), vmem(s_shape, F32),
            vmem((8, 128), U32),
            vmem((9, fill_rows // 2, D2), U32),
            vmem((D, D), BF16), vmem((D2, D), U32),
        ],
        compiler_params=pltpu.CompilerParams(
            dimension_semantics=("arbitrary",),
            vmem_limit_bytes=100 * 1024 * 1024,
            disable_bounds_checks=True,
        ),
    )(x.reshape(B, 2, T2, D), w_q, w_k, w_v, w_ao, w_up, dw, w_dn, w_merge)
    return out.reshape(B, T, D)
```
